```python
import jax
import jax.numpy as jnp

def _softmax(x, axis=-1):
    return jax.nn.softmax(x, axis=axis)
def _gelu(x):
    return jax.nn.gelu(x, approximate=True)
def _silu(x):
    return jax.nn.silu(x)
def _sigmoid(x):
    return jax.nn.sigmoid(x)
def _layernorm(x, axis=-1, eps=1e-5):
    m = jnp.mean(x, axis=axis, keepdims=True)
    v = jnp.var(x, axis=axis, keepdims=True)
    return (x - m) / jnp.sqrt(v + eps)
def _scatter_add(tgt, idx, src, axis=0):
    return tgt.at[idx].add(src)
def _segment_sum(src, seg, n):
    return jax.ops.segment_sum(src, seg, n)
class _Rng:
    def __init__(self, key):
        self._k = key
    def _next(self):
        self._k, sub = jax.random.split(self._k)
        return sub
    def normal(self, shape):
        return jax.random.normal(self._next(), shape, dtype=jnp.bfloat16)
    def randint(self, lo, hi, shape):
        return jax.random.randint(self._next(), shape, lo, hi, dtype=jnp.int32)
    def uniform(self, shape, lo=0.0, hi=1.0):
        return jax.random.uniform(self._next(), shape, jnp.bfloat16, lo, hi)
    def permutation(self, n):
        return jax.random.permutation(self._next(), n)


kernel_name = 'concat_heads__gqa_block_cached__gqa_block_cached__near_ridge'

def _fwd_setup_inputs():
    _rng = _Rng(jax.random.key(int.from_bytes(__import__("os").urandom(4), "little")))
    _w = (lambda a: (lambda t: t.astype(jnp.bfloat16) if jnp.issubdtype(t.dtype, jnp.floating) else t)(jnp.asarray(a)))
    def _A_setup():
        B, Sq, D = 16, 112, 640
        Hq, Hkv, Sk, Dh = 32, 32, 512, 128
        assert Hq % Hkv == 0, (Hq, Hkv)
        return {
            "x": _w((lambda *s: _rng.normal(s) * 0.05)(B, Sq, D)),
            "k_cache": _w((lambda *s: _rng.normal(s) * 0.05)(B, Hkv, Sk, Dh)),
            "v_cache": _w((lambda *s: _rng.normal(s) * 0.05)(B, Hkv, Sk, Dh)),
            "wq": _w((lambda *s: _rng.normal(s) * 0.05)(D, Hq * Dh) * (D ** -0.5)),
            "wo": _w((lambda *s: _rng.normal(s) * 0.05)(Hq * Dh, D) * ((Hq * Dh) ** -0.5)),
        }
    _A_in = _A_setup()

    def _B_setup():
        B, Sq, D = 16, 112, 640
        Hq, Hkv, Sk, Dh = 32, 32, 512, 128
        assert Hq % Hkv == 0, (Hq, Hkv)
        return {
            "x": _w((lambda *s: _rng.normal(s) * 0.05)(B, Sq, D)),
            "k_cache": _w((lambda *s: _rng.normal(s) * 0.05)(B, Hkv, Sk, Dh)),
            "v_cache": _w((lambda *s: _rng.normal(s) * 0.05)(B, Hkv, Sk, Dh)),
            "wq": _w((lambda *s: _rng.normal(s) * 0.05)(D, Hq * Dh) * (D ** -0.5)),
            "wo": _w((lambda *s: _rng.normal(s) * 0.05)(Hq * Dh, D) * ((Hq * Dh) ** -0.5)),
        }
    _B_in = _B_setup()

    return {
        "A_x": _A_in["x"],
        "A_k_cache": _A_in["k_cache"],
        "A_v_cache": _A_in["v_cache"],
        "A_wq": _A_in["wq"],
        "A_wo": _A_in["wo"],
        "B_x": _B_in["x"],
        "B_k_cache": _B_in["k_cache"],
        "B_v_cache": _B_in["v_cache"],
        "B_wq": _B_in["wq"],
        "B_wo": _B_in["wo"],
    }

def _fwd_reference(A_x, A_k_cache, A_v_cache, A_wq, A_wo, B_x, B_k_cache, B_v_cache, B_wq, B_wo):
    def _A_ref(x, k_cache, v_cache, wq, wo):
        B, Sq, D = x.shape
        Hq, Dh = 32, 128
        Hkv = k_cache.shape[1]
        rep = Hq // Hkv
        q = (lambda x, *d: x.transpose(*d))((x @ wq).reshape(B, Sq, Hq, Dh), 0, 2, 1, 3)
        k = jnp.repeat(k_cache, rep, axis=1)
        v = jnp.repeat(v_cache, rep, axis=1)
        scores = jnp.einsum("bhqd,bhkd->bhqk", q, k) * (Dh ** -0.5)
        p = _softmax(scores, axis=-1)
        o = jnp.einsum("bhqk,bhkd->bhqd", p, v)
        return (lambda x, *d: x.transpose(*d))(o, 0, 2, 1, 3).reshape(B, Sq, Hq * Dh) @ wo

    def _B_ref(x, k_cache, v_cache, wq, wo):
        B, Sq, D = x.shape
        Hq, Dh = 32, 128
        Hkv = k_cache.shape[1]
        rep = Hq // Hkv
        q = (lambda x, *d: x.transpose(*d))((x @ wq).reshape(B, Sq, Hq, Dh), 0, 2, 1, 3)
        k = jnp.repeat(k_cache, rep, axis=1)
        v = jnp.repeat(v_cache, rep, axis=1)
        scores = jnp.einsum("bhqd,bhkd->bhqk", q, k) * (Dh ** -0.5)
        p = _softmax(scores, axis=-1)
        o = jnp.einsum("bhqk,bhkd->bhqd", p, v)
        return (lambda x, *d: x.transpose(*d))(o, 0, 2, 1, 3).reshape(B, Sq, Hq * Dh) @ wo

    a = _A_ref(A_x, A_k_cache, A_v_cache, A_wq, A_wo)
    b = _B_ref(B_x, B_k_cache, B_v_cache, B_wq, B_wo)
    return jnp.concatenate([a, b], axis=-1)


def setup_inputs():
    _inp = _fwd_setup_inputs()
    _gk = jax.random.fold_in(jax.random.key(int.from_bytes(__import__("os").urandom(4), "little")), 2**31 - 1)
    _shapes = [[16, 112, 1280]]
    _dtypes = ['bfloat16']
    _gks = jax.random.split(_gk, len(_shapes))
    _gs = [jax.random.normal(k, s, dtype=jnp.dtype(d)) * 0.05 for k, s, d in zip(_gks, _shapes, _dtypes)]
    _inp["grad_out"] = _gs[0]
    return _inp

def reference(A_x, A_k_cache, A_v_cache, A_wq, A_wo, B_x, B_k_cache, B_v_cache, B_wq, B_wo, grad_out):
    _const = dict()
    def _f(*_d):
        return _fwd_reference(**{'A_x': _d[0], 'A_k_cache': _d[1], 'A_v_cache': _d[2], 'A_wq': _d[3], 'A_wo': _d[4], 'B_x': _d[5], 'B_k_cache': _d[6], 'B_v_cache': _d[7], 'B_wq': _d[8], 'B_wo': _d[9], **_const})
    _out, _vjp = jax.vjp(_f, A_x, A_k_cache, A_v_cache, A_wq, A_wo, B_x, B_k_cache, B_v_cache, B_wq, B_wo)
    _grads = _vjp(grad_out)
    _out0 = jnp.asarray(_out)
    return (_out0, *[jnp.asarray(_g) for _g in _grads])
```

```python
import functools
import jax, jax.numpy as jnp
from jax import lax
from jax.experimental import pallas as pl
from jax.experimental.pallas import tpu as pltpu

NAME = "concat_heads_gqa_fwd_bwd"
B, SQ, D, H, SK, DH = 16, 112, 640, 32, 512, 128
T = B * SQ
F32, BF16, U32 = jnp.float32, jnp.bfloat16, jnp.uint32
NN = (((1,), (0,)), ((), ()))
NT = (((1,), (1,)), ((), ()))
TN = (((0,), (0,)), ((), ()))
SCALE = DH ** -0.5
LOG2E = 1.4426950408889634


def kernel(xa, ka, va, wqa, woa, xb, kb, vb, wqb, wob, go,
           out, dxa, dka, dva, dwqa, dwoa, dxb, dkb, dvb, dwqb, dwob,
           *scr, G, order, dwmode):
    NS = H // G
    W = G * DH
    it = iter(scr)
    kbuf, vbuf = next(it), next(it)
    dkbufs = [next(it) for _ in range(G)]
    dvbufs = [next(it) for _ in range(G)]
    wqbuf, wobuf, dwqbuf, dwobuf = next(it), next(it), next(it), next(it)
    xbuf, gobuf, obuf, dxbuf = next(it), next(it), next(it), next(it)
    out_acc, dx_acc = next(it), next(it)
    q_s, do_s, o_s, dq_s = next(it), next(it), next(it), next(it)
    sem_in, sem_out, sem_act = next(it), next(it), next(it)

    i = pl.program_id(0)
    r = i // NS
    slot = i % 2
    br = ((xa, ka, va, wqa, woa, dxa, dka, dva, dwqa, dwoa),
          (xb, kb, vb, wqb, wob, dxb, dkb, dvb, dwqb, dwob))

    def in_copies(rr, hp, s):
        _, k, v, wq, wo = br[rr][:5]
        c0 = pl.multiple_of(hp * W, W)
        return [
            pltpu.make_async_copy(wq.at[:, pl.ds(c0, W)], wqbuf.at[s], sem_in.at[s, 0]),
            pltpu.make_async_copy(wo.at[pl.ds(c0, W), :], wobuf.at[s], sem_in.at[s, 1]),
            pltpu.make_async_copy(k.at[:, pl.ds(hp * G, G)], kbuf.at[s], sem_in.at[s, 2]),
            pltpu.make_async_copy(v.at[:, pl.ds(hp * G, G)], vbuf.at[s], sem_in.at[s, 3]),
        ]

    def dkv_copies(rr, hp, s, g):
        dk, dv = br[rr][6:8]
        return [
            pltpu.make_async_copy(dkbufs[g].at[s], dk.at[:, hp * G + g], sem_out.at[s, 2 + 2 * g]),
            pltpu.make_async_copy(dvbufs[g].at[s], dv.at[:, hp * G + g], sem_out.at[s, 3 + 2 * g]),
        ]

    def dw_copies(rr, hp, s):
        dwq, dwo = br[rr][8:10]
        c0 = pl.multiple_of(hp * W, W)
        return [
            pltpu.make_async_copy(dwqbuf.at[s], dwq.at[:, pl.ds(c0, W)], sem_out.at[s, 0]),
            pltpu.make_async_copy(dwobuf.at[s], dwo.at[pl.ds(c0, W), :], sem_out.at[s, 1]),
        ]

    def act_in(rr):
        return [
            pltpu.make_async_copy(br[rr][0], xbuf.at[rr], sem_act.at[rr, 0]),
            pltpu.make_async_copy(go.at[:, pl.ds(rr * D, D)], gobuf.at[rr], sem_act.at[rr, 1]),
        ]

    def act_out(rr):
        return [
            pltpu.make_async_copy(obuf.at[rr], out.at[:, pl.ds(rr * D, D)], sem_act.at[rr, 2]),
            pltpu.make_async_copy(dxbuf.at[rr], br[rr][5], sem_act.at[rr, 3]),
        ]

    def for_step(step, fn):
        for rr in range(2):
            @pl.when(jnp.logical_and(step >= rr * NS, step < (rr + 1) * NS))
            def _():
                fn(rr, step - rr * NS)

    @pl.when(i == 0)
    def _():
        for c in act_in(0):
            c.start()
        for c in in_copies(0, 0, 0):
            c.start()

    for c in in_copies(0, 0, slot):
        c.wait()
    for rr in range(2):
        @pl.when(i == rr * NS)
        def _():
            for c in act_in(rr):
                c.wait()

    @pl.when(i >= 2)
    def _():
        for g in range(G):
            for c in dkv_copies(0, 0, slot, g):
                c.wait()
        for c in dw_copies(0, 0, slot):
            c.wait()

    for_step(i + 1, lambda rr, hp: [c.start() for c in in_copies(rr, hp, 1 - slot)])

    @pl.when(i == 1)
    def _():
        for c in act_in(1):
            c.start()

    first = (i % NS) == 0
    last = (i % NS) == NS - 1
    x = xbuf.at[r]
    gos = gobuf.at[r]
    wq = wqbuf[slot]
    wo = wobuf[slot]
    qq = lax.dot_general(x[...], wq, NN, preferred_element_type=F32).astype(BF16)
    dd = lax.dot_general(gos[...], wo, NT, preferred_element_type=F32).astype(BF16)
    for g in range(G):
        q_s[g] = qq[:, g * DH:(g + 1) * DH]
        do_s[g] = dd[:, g * DH:(g + 1) * DH]

    k32 = kbuf.bitcast(U32)
    v32 = vbuf.bitcast(U32)
    n_units = G * B
    st = [dict() for _ in range(n_units)]
    rows = lambda b: pl.ds(b * SQ, SQ)
    getk = lambda g, b: pltpu.bitcast(k32[slot, b, g], BF16)
    getv = lambda g, b: pltpu.bitcast(v32[slot, b, g], BF16)

    def S(u):
        g, b = divmod(u, B)
        q = q_s[g, rows(b), :]
        s = lax.dot_general(q, getk(g, b), NT, preferred_element_type=F32) * (SCALE * LOG2E)
        m = jnp.max(s, axis=-1, keepdims=True)
        e = jnp.exp2(s - m)
        l = jnp.sum(e, axis=-1, keepdims=True)
        rc = pl.reciprocal(l, approx=True)
        rc = rc * (2.0 - l * rc)
        st[u].update(e=e, eb=e.astype(BF16), r=rc)
    def P(u):
        g, b = divmod(u, B)
        dp = lax.dot_general(do_s[g, rows(b), :], getv(g, b), NT, preferred_element_type=F32)
        st[u].update(dp=dp)
    def O(u):
        g, b = divmod(u, B)
        o = lax.dot_general(st[u]['eb'], getv(g, b), NN, preferred_element_type=F32) * st[u]['r']
        o_s[rows(b), g * DH:(g + 1) * DH] = o.astype(BF16)
        st[u].update(o=o)
    def V(u):
        g, b = divmod(u, B)
        dor = (do_s[g, rows(b), :].astype(F32) * st[u]['r']).astype(BF16)
        dv = lax.dot_general(st[u]['eb'], dor, TN, preferred_element_type=F32)
        dvbufs[g][slot, b] = dv.astype(BF16)
    def DS(u):
        if 'ds' in st[u]: return
        g, b = divmod(u, B)
        e, dp = st[u]['e'], st[u]['dp']
        delta = jnp.sum(st[u]['o'] * do_s[g, rows(b), :].astype(F32), axis=-1, keepdims=True)
        st[u]['ds'] = (e * (dp - delta)).astype(BF16)
    def Q(u):
        DS(u)
        g, b = divmod(u, B)
        dq = lax.dot_general(st[u]['ds'], getk(g, b), NN, preferred_element_type=F32) * (st[u]['r'] * SCALE)
        dq_s[rows(b), g * DH:(g + 1) * DH] = dq.astype(BF16)
    def K(u):
        DS(u)
        g, b = divmod(u, B)
        qr = (q_s[g, rows(b), :].astype(F32) * (st[u]['r'] * SCALE)).astype(BF16)
        dk = lax.dot_general(st[u]['ds'], qr, TN, preferred_element_type=F32)
        dkbufs[g][slot, b] = dk.astype(BF16)
        if b == B - 1:
            for_step(i, lambda rr, hp: [c.start() for c in dkv_copies(rr, hp, slot, g)])
        st[u].clear()
    fns = dict(S=S, P=P, O=O, V=V, Q=Q, K=K)
    maxlag = max(l for _, l in order)
    for t in range(n_units + maxlag):
        for name, lag in order:
            u = t - lag
            if 0 <= u < n_units:
                fns[name](u)

    o = o_s[...]
    dq = dq_s[...]
    acc = jnp.where(first, 0.0, out_acc[...]) + lax.dot_general(o, wo, NN, preferred_element_type=F32)
    out_acc[...] = acc
    obuf[r] = acc.astype(BF16)
    acc = jnp.where(first, 0.0, dx_acc[...]) + lax.dot_general(dq, wq, NT, preferred_element_type=F32)
    dx_acc[...] = acc
    dxbuf[r] = acc.astype(BF16)
    for rr in range(2):
        @pl.when(i == (rr + 1) * NS - 1)
        def _():
            for c in act_out(rr):
                c.start()
    dwqbuf[slot] = lax.dot_general(dq, x[...], TN, preferred_element_type=F32).astype(BF16).T
    dwobuf[slot] = lax.dot_general(o, gos[...], TN, preferred_element_type=F32).astype(BF16)
    for_step(i, lambda rr, hp: [c.start() for c in dw_copies(rr, hp, slot)])

    @pl.when(i == 2 * NS - 1)
    def _():
        for s in range(2):
            for g in range(G):
                for c in dkv_copies(0, 0, s, g):
                    c.wait()
            for c in dw_copies(0, 0, s):
                c.wait()
        for rr in range(2):
            for c in act_out(rr):
                c.wait()


def run_full(xa, ka, va, wqa, woa, xb, kb, vb, wqb, wob, go, G=1, order="S0 P0 O1 V1 Q2 K2", dwmode="tn"):
    order = [(w[0], int(w[1:])) for w in order.split()]
    W = G * DH
    anyspec = pl.BlockSpec(memory_space=pl.ANY)
    sds = lambda s: jax.ShapeDtypeStruct(s, BF16)
    br_out = [sds((T, D)), sds(ka.shape), sds(va.shape), sds(wqa.shape), sds(woa.shape)]
    V = pltpu.VMEM
    scratch = ([V((2, B, G, SK, DH), BF16)] * 2 + [V((2, B, SK, DH), BF16)] * (2 * G)
               + [V((2, D, W), BF16), V((2, W, D), BF16), V((2, D, W), BF16), V((2, W, D), BF16)]
               + [V((2, T, D), BF16)] * 4 + [V((T, D), F32)] * 2
               + [V((G, T, DH), BF16)] * 2 + [V((T, W), BF16)] * 2
               + [pltpu.SemaphoreType.DMA((2, 4)), pltpu.SemaphoreType.DMA((2, 2 + 2 * G)),
                  pltpu.SemaphoreType.DMA((2, 4))])
    outs = pl.pallas_call(
        functools.partial(kernel, G=G, order=order, dwmode=dwmode),
        grid=(2 * H // G,),
        in_specs=[anyspec] * 11,
        out_specs=[anyspec] * 11,
        out_shape=[sds((T, 2 * D))] + br_out + br_out,
        scratch_shapes=scratch,
        compiler_params=pltpu.CompilerParams(dimension_semantics=("arbitrary",), vmem_limit_bytes=110 * 2**20),
        name=NAME,
    )(xa.reshape(T, D), ka, va, wqa, woa, xb.reshape(T, D), kb, vb, wqb, wob, go.reshape(T, 2 * D))
    o = list(outs)
    o[0] = o[0].reshape(B, SQ, 2 * D)
    o[1] = o[1].reshape(B, SQ, D)
    o[6] = o[6].reshape(B, SQ, D)
    return tuple(o)


@jax.jit
def pallas_concat_heads__gqa_block_cached__gqa_block_cached__near_ridge_kernel(
    A_x, A_k_cache, A_v_cache, A_wq, A_wo, B_x, B_k_cache, B_v_cache, B_wq, B_wo, grad_out
):
    return run_full(A_x, A_k_cache, A_v_cache, A_wq, A_wo, B_x, B_k_cache, B_v_cache, B_wq, B_wo,
                    grad_out, G=2)
```

```python
import functools
import jax, jax.numpy as jnp
from jax import lax
from jax.experimental import pallas as pl
from jax.experimental.pallas import tpu as pltpu

NAME = "concat_heads_gqa_fwd_bwd"
B, SQ, D, H, SK, DH = 16, 112, 640, 32, 512, 128
T = B * SQ
TH = T // 2
G = 2
W = G * DH
NS = H // G
NB = B // 2
DP = 256
DC = D - 2 * DP
DHF = D // 2
F32, BF16, U32 = jnp.float32, jnp.bfloat16, jnp.uint32
NN = (((1,), (0,)), ((), ()))
NT = (((1,), (1,)), ((), ()))
TN = (((0,), (0,)), ((), ()))
SCALE = DH ** -0.5
LOG2E = 1.4426950408889634
BORD = (0, 2, 6, 5, 3, 4, 1)


def combos(z11, z12, z21, z22):
    f11, f12, f21, f22 = (z.astype(F32) for z in (z11, z12, z21, z22))
    return [c.astype(BF16) for c in
            (f11 + f22, f21 + f22, z11, z22, f11 + f12, f21 - f11, f12 - f22)]


def recombine(m):
    c11 = m[0] + m[3] - m[4] + m[6]
    c12 = m[2] + m[4]
    c21 = m[1] + m[3]
    c22 = m[0] - m[1] + m[2] + m[5]
    return c11, c12, c21, c22


def rt(x):
    return x.astype(F32).astype(BF16)


def upk(x):
    return pltpu.bitcast(x, BF16)


def kernel(xa, ka, va, wqa, woa, xb, kb, vb, wqb, wob, go,
           out, dxa, dka, dva, dwqa, dwoa, dxb, dkb, dvb, dwqb, dwob,
           kbuf, vbuf, dkbuf, dvbuf, wqbuf, wobuf, dwqbuf, dwobuf,
           xbuf, gobuf, obuf, dxbuf,
           xc, gc, xt, gt, om, ol, dm, dl, q_s, do_s, oc, dqc, eb_s,
           sem_in, sem_out, sem_act, *, sched, kvsplit, morder, ebf, cacc, yorder, rchunk, nsteps):
    i = pl.program_id(0)
    r = i // NS
    slot = i % 2
    br = ((xa, ka, va, wqa, woa, dxa, dka, dva, dwqa, dwoa),
          (xb, kb, vb, wqb, wob, dxb, dkb, dvb, dwqb, dwob))
    col0 = lambda hp: hp * W if isinstance(hp, int) else pl.multiple_of(hp * W, W)
    kvg = [0] + list(kvsplit) + [B]

    def w_in(rr, hp, s):
        wq, wo = br[rr][3:5]
        return [pltpu.make_async_copy(wq.at[:, pl.ds(col0(hp), W)], wqbuf.at[s], sem_in.at[s, 0]),
                pltpu.make_async_copy(wo.at[pl.ds(col0(hp), W), :], wobuf.at[s], sem_in.at[s, 1])]

    def kv_in(rr, hp, s, g):
        k, v = br[rr][1:3]
        bs = pl.ds(kvg[g], kvg[g + 1] - kvg[g])
        return [pltpu.make_async_copy(k.at[bs, pl.ds(hp * G, G)], kbuf.at[s, bs], sem_in.at[s, 2 + 2 * g]),
                pltpu.make_async_copy(v.at[bs, pl.ds(hp * G, G)], vbuf.at[s, bs], sem_in.at[s, 3 + 2 * g])]

    def all_in(rr, hp, s):
        return w_in(rr, hp, s) + [c for g in range(len(kvg) - 1) for c in kv_in(rr, hp, s, g)]

    def dkv_out(rr, hp, s, which, bs):
        src, dst = (dkbuf, dvbuf)[which], br[rr][6 + which]
        return pltpu.make_async_copy(src.at[s, bs], dst.at[bs, pl.ds(hp * G, G)], sem_out.at[s, which])

    def dw_out(rr, hp, s):
        dwq, dwo = br[rr][8:10]
        return [pltpu.make_async_copy(dwqbuf.at[s], dwq.at[:, pl.ds(col0(hp), W)], sem_out.at[s, 2]),
                pltpu.make_async_copy(dwobuf.at[s], dwo.at[pl.ds(col0(hp), W), :], sem_out.at[s, 3])]

    def wait_out(s):
        for which in range(2):
            dkv_out(0, 0, s, which, pl.ds(0, B)).wait()
        for c in dw_out(0, 0, s):
            c.wait()

    def act_in(rr):
        return [pltpu.make_async_copy(br[rr][0], xbuf, sem_act.at[0]),
                pltpu.make_async_copy(go.at[:, pl.ds(rr * D, D)], gobuf, sem_act.at[1])]

    def act_out(rr, which, rows):
        if which == 0:
            return pltpu.make_async_copy(obuf.at[rr, rows], out.at[rows, pl.ds(rr * D, D)], sem_act.at[2 + 2 * rr])
        return pltpu.make_async_copy(dxbuf.at[rr, rows], br[rr][5].at[rows], sem_act.at[3 + 2 * rr])

    def for_step(step, fn):
        for rr in range(2):
            @pl.when(jnp.logical_and(step >= rr * NS, step < min(nsteps, (rr + 1) * NS)))
            def _():
                fn(rr, step - rr * NS)

    @pl.when(i == 0)
    def _():
        for c in act_in(0) + w_in(0, 0, 0):
            c.start()

    first = (i % NS) == 0

    @pl.when(first)
    def _():
        for c in act_in(0):
            c.wait()

        @pl.when(i == 0)
        def _():
            for g in range(len(kvg) - 1):
                for c in kv_in(0, 0, 0, g):
                    c.start()

        def natural(src, cmb, be):
            c32 = cmb.bitcast(U32)
            for p in range(0, SQ, rchunk):
                n_r = min(rchunk, SQ - p)
                r1, r2 = pl.ds(2 * be * SQ + p, n_r), pl.ds((2 * be + 1) * SQ + p, n_r)
                ro, rh = pl.ds(be * SQ + p, n_r), pl.ds((be * SQ + p) // 2, n_r // 2)
                for c in range(2):
                    f = lambda rr, d: src[rr, pl.ds(d * DP + c * 128, 128)]
                    cs = combos(f(r1, 0), f(r2, 0), f(r1, 1), f(r2, 1))
                    for n in (0, 1, 4, 5, 6):
                        cmb[2 * n + c, ro, :] = cs[n]
                    c32[4 + c, rh, :] = pltpu.bitcast(f(r1, 0), U32)
                    c32[6 + c, rh, :] = pltpu.bitcast(f(r2, 1), U32)
                c32[14, rh, :] = pltpu.bitcast(src[r1, pl.ds(2 * DP, DC)], U32)
                c32[15, rh, :] = pltpu.bitcast(src[r2, pl.ds(2 * DP, DC)], U32)

        def transposed(src, cmt, c):
            c32 = cmt.bitcast(U32)
            def tile_t(t, d):
                lo, hi = c * 128, (c + 1) * 128
                parts = []
                while lo < hi:
                    be, off = divmod(lo, SQ)
                    n = min(hi - lo, SQ - off)
                    parts.append(src[pl.ds((2 * be + t) * SQ + off, n), pl.ds(d * 128, 128)])
                    lo += n
                return jnp.concatenate(parts, axis=0).T
            for d in range(D // 128):
                z1, z2 = tile_t(0, d), tile_t(1, d)
                cs = combos(z1[:64], z2[:64], z1[64:], z2[64:])
                for n in (0, 1, 4, 5, 6):
                    cmt[n, c, pl.ds(d * 64, 64), :] = cs[n]
                c32[2, c, pl.ds(d * 32, 32), :] = pltpu.bitcast(z1, U32)[:32]
                c32[3, c, pl.ds(d * 32, 32), :] = pltpu.bitcast(z2, U32)[32:]

        for src, cmb, cmt in ((xbuf, xc, xt), (gobuf, gc, gt)):
            for be in range(NB):
                if be < TH // 128:
                    transposed(src, cmt, be)
                natural(src, cmb, be)

    if nsteps > NS:
        @pl.when(i == 1)
        def _():
            for c in act_in(1):
                c.start()

    for c in w_in(0, 0, slot) + kv_in(0, 0, slot, 0):
        c.wait()

    @pl.when(i >= 2)
    def _():
        wait_out(slot)

    wq = wqbuf[slot]
    wo = wobuf[slot]
    fq = lambda d, j: wq[d * DP:(d + 1) * DP, j * DH:(j + 1) * DH]
    fo = lambda j, d: wo[j * DH:(j + 1) * DH, d * DP:(d + 1) * DP]
    wqc = combos(fq(0, 0), fq(1, 0), fq(0, 1), fq(1, 1))
    woc = combos(fo(0, 0), fo(0, 1), fo(1, 0), fo(1, 1))
    wql = wq[2 * DP:, :]
    wol = wo[:, 2 * DP:]

    k32, v32, q32, do32, oc32, dqc32, xc32, gc32, xt32, gt32 = (
        z.bitcast(U32) for z in (kbuf, vbuf, q_s, do_s, oc, dqc, xc, gc, xt, gt))
    eb32 = eb_s.bitcast(U32)
    n_units = G * B
    st = [dict() for _ in range(n_units)]
    ov, dqv = {}, {}
    hrow = lambda be: pl.ds(be * SQ // 2, SQ // 2)
    getk = lambda b, j: upk(k32[slot, b, j])
    getv = lambda b, j: upk(v32[slot, b, j])
    getq = lambda b, j: upk(q32[j, b % 2, hrow(b // 2), :])
    getdo = lambda b, j: upk(do32[j, b % 2, hrow(b // 2), :])

    def proj_in(be, c32, wc, wl, dn, dst, mul):
        get = lambda n: upk(c32[n, hrow(be), :])
        lo = [lax.dot_general(get(14 + t), wl, dn, preferred_element_type=F32) for t in range(2)]
        m = [None] * 7
        for n in morder:
            lhs = jnp.concatenate([get(2 * BORD[n]), get(2 * BORD[n] + 1)], axis=1)
            m[n] = lax.dot_general(lhs, wc[n], dn, preferred_element_type=F32)
        cjt = recombine(m)
        for t in range(2):
            for j in range(2):
                val = cjt[2 * j + t] + lo[t][:, j * DH:(j + 1) * DH]
                if mul is not None:
                    val = val * mul
                dst[j, t, pl.ds(be * SQ, SQ), :] = val.astype(BF16)

    def proj_out(be, vals, cst, c32, wc, wl, dn, macc, lacc, stage, which):
        z = [[vals.pop((2 * be + t, j)) for j in range(2)] for t in range(2)]
        cs = combos(z[0][0], z[0][1], z[1][0], z[1][1]) + [z[0][1].astype(BF16), z[1][0].astype(BF16)]
        ro = pl.ds(be * SQ, SQ)
        for n in range(9):
            cst[n, ro, :] = cs[n]
        get = lambda n: upk(c32[n, hrow(be), :])
        half = (lambda j: wl[j * DH:(j + 1) * DH, :]) if dn is NN else (lambda j: wl[:, j * DH:(j + 1) * DH])
        left = lambda n0, n1: (lax.dot_general(get(n0), half(0), dn, preferred_element_type=F32)
                               + lax.dot_general(get(n1), half(1), dn, preferred_element_type=F32))
        if cacc == 0:
            m = [None] * 7
            for n in yorder:
                m[n] = jnp.where(first, 0.0, macc[n, ro, :]) + lax.dot_general(get(n), wc[BORD[n]], dn, preferred_element_type=F32)
                macc[n, ro, :] = m[n]
            c = recombine(m)
        elif cacc == 1:
            m = [None] * 7
            for n in yorder:
                m[n] = lax.dot_general(get(n), wc[BORD[n]], dn, preferred_element_type=F32)
            c = list(recombine(m))
            for n in range(4):
                c[n] = c[n] + jnp.where(first, 0.0, macc[n, ro, :])
                macc[n, ro, :] = c[n]
        else:
            cc = []
            for h in range(2):
                wh = (lambda w: w[:, h * 128:(h + 1) * 128]) if dn is NN else (lambda w: w[h * 128:(h + 1) * 128, :])
                m = [None] * 7
                for n in yorder:
                    m[n] = lax.dot_general(get(n), wh(wc[BORD[n]]), dn, preferred_element_type=F32)
                c = list(recombine(m))
                for n in range(4):
                    c[n] = c[n] + jnp.where(first, 0.0, macc[n, ro, h * 128:(h + 1) * 128])
                    macc[n, ro, h * 128:(h + 1) * 128] = c[n]
                cc.append(c)
            c = [jnp.concatenate([cc[0][n], cc[1][n]], axis=1) for n in range(4)]
        for t, (n0, n1) in enumerate(((2, 7), (8, 3))):
            lo = jnp.where(first, 0.0, lacc[t, ro, :]) + left(n0, n1)
            lacc[t, ro, :] = lo
            row = jnp.concatenate([c[2 * t], c[2 * t + 1], lo], axis=1)
            stage[r, pl.ds((2 * be + t) * SQ, SQ), :] = row.astype(BF16)
        for rr in range(2):
            @pl.when(i == (rr + 1) * NS - 1)
            def _():
                act_out(rr, which, pl.ds(2 * be * SQ, 2 * SQ)).start()

    def S(u):
        b, j = divmod(u, G)
        s = lax.dot_general(getq(b, j), getk(b, j), NT, preferred_element_type=F32)
        m = jnp.max(s, axis=-1, keepdims=True)
        e = jnp.exp2(s - m)
        l = jnp.sum(e, axis=-1, keepdims=True)
        rcp = pl.reciprocal(l, approx=True)
        rcp = rcp * (2.0 - l * rcp)
        if ebf:
            for c in range(4):
                eb_s[u % 4, c] = e[:, c * 128:(c + 1) * 128].astype(BF16)
            geteb = lambda: jnp.concatenate([upk(eb32[u % 4, c]) for c in range(4)], axis=1)
            st[u].update(geteb=geteb, gete=lambda: geteb().astype(F32), r=rcp)
        else:
            eb = e.astype(BF16)
            st[u].update(geteb=lambda: eb, gete=lambda: e, r=rcp)
    def P(u):
        b, j = divmod(u, G)
        st[u]['dp'] = lax.dot_general(getdo(b, j), getv(b, j), NT, preferred_element_type=F32)
    def O(u):
        b, j = divmod(u, G)
        o = lax.dot_general(st[u]['geteb'](), getv(b, j), NN, preferred_element_type=F32) * st[u]['r']
        dof = getdo(b, j).astype(F32)
        st[u]['delta'] = jnp.sum(o * dof, axis=-1, keepdims=True)
        st[u]['dor'] = (dof * st[u]['r']).astype(BF16)
        ov[b, j] = o
    def flush(u, which):
        if u % 4 == 3:
            for_step(i, lambda rr, hp: dkv_out(rr, hp, slot, which, pl.ds(u // 4 * 2, 2)).start())
    def V(u):
        b, j = divmod(u, G)
        dv = lax.dot_general(st[u]['geteb'](), st[u]['dor'], TN, preferred_element_type=F32)
        dvbuf[slot, b, j] = dv.astype(BF16)
        flush(u, 1)
    def Q(u):
        b, j = divmod(u, G)
        st[u]['ds'] = (st[u]['gete']() * (st[u]['dp'] - st[u]['delta'])).astype(BF16)
        dqv[b, j] = lax.dot_general(st[u]['ds'], getk(b, j), NN, preferred_element_type=F32) * (st[u]['r'] * SCALE)
    def K(u):
        b, j = divmod(u, G)
        qr = (getq(b, j).astype(F32) * (st[u]['r'] * (1.0 / LOG2E))).astype(BF16)
        dk = lax.dot_general(st[u]['ds'], qr, TN, preferred_element_type=F32)
        dkbuf[slot, b, j] = dk.astype(BF16)
        flush(u, 0)
        st[u].clear()

    def proj_w(c32, zt32):
        m = []
        for n in range(7):
            rhs = upk(c32[BORD[n]])
            lhs = jnp.concatenate([upk(zt32[n, c]) for c in range(TH // 128)], axis=1)
            m.append(lax.dot_general(lhs, rhs, NN, preferred_element_type=F32))
        c = recombine(m)
        top = jnp.concatenate([c[0], c[1]], axis=1)
        bot = jnp.concatenate([c[2], c[3]], axis=1)
        rows = [z[d * 64:(d + 1) * 64] for d in range(D // 128) for z in (top, bot)]
        return jnp.concatenate(rows, axis=0).astype(BF16)
    def WO(_):
        dwobuf[slot] = proj_w(oc32, gt32).T
    def WQ(_):
        dwqbuf[slot] = proj_w(dqc32, xt32)
    def XQ(c):
        proj_in(c, xc32, wqc, wql, NN, q_s, SCALE * LOG2E)
    def XO(c):
        proj_in(c, gc32, woc, wol, NT, do_s, None)
    def YO(c):
        proj_out(c, ov, oc, oc32, woc, wol, NN, om, ol, obuf, 0)
    def YQ(c):
        proj_out(c, dqv, dqc, dqc32, wqc, wql, NT, dm, dl, dxbuf, 1)
    def WAIT(g):
        for c in kv_in(0, 0, slot, g):
            c.wait()
        if g == len(kvg) - 2:
            @pl.when(i == 0)
            def _():
                for c in all_in(0, 1, 1):
                    c.start()

    if len(kvg) == 2 and nsteps > 1:
        @pl.when(i == 0)
        def _():
            for c in all_in(0, 1, 1):
                c.start()

    fns = dict(S=S, P=P, O=O, V=V, Q=Q, K=K, XQ=XQ, XO=XO, YO=YO, YQ=YQ, WO=WO, WQ=WQ, WAIT=WAIT)
    for name, idx in sched:
        fns[name](idx)

    for_step(i, lambda rr, hp: [c.start() for c in dw_out(rr, hp, slot)])
    for_step(i + 2, lambda rr, hp: [c.start() for c in all_in(rr, hp, slot)])

    @pl.when(i == nsteps - 1)
    def _():
        for s in range(min(2, nsteps)):
            wait_out(s)
        for rr in range(nsteps // NS):
            for which in range(2):
                act_out(rr, which, pl.ds(0, T)).wait()


def build_sched(order, extra, moves, kvsplit, waits):
    order = [(w[0], int(w[1:])) for w in order.split()]
    n_units = G * B
    ex = []
    for w in extra.split():
        name, rest = w.split('@')
        off, after = rest.split('/')
        ex.append((name, int(off), after))
    sched = []
    for t in range(-16, n_units + 16):
        pos = [('^', None)] + [(nm, t - lag) for nm, lag in order]
        for nm, u in pos:
            if u is not None and 0 <= u < n_units:
                sched.append((nm, u))
            for en, off, after in ex:
                if after == nm and (t - off) % 4 == 0 and 0 <= (t - off) // 4 < NB:
                    sched.append((en, (t - off) // 4))
    sched += [('WO', 0), ('WQ', 0)]
    pa = lambda z: (z.rstrip('0123456789'), int(z[len(z.rstrip('0123456789')):]))
    for mv in moves.split():
        a, b = map(pa, mv.split('>'))
        sched.remove(a)
        sched.insert(sched.index(b) + 1, a)
    for g, w in enumerate(waits.split()):
        sched.insert(sched.index(pa(w)) + 1, ('WAIT', g + 1))
    pos = {it: n for n, it in enumerate(sched)}
    assert len(pos) == len(sched) == 6 * n_units + 4 * NB + 2 + len(kvsplit)
    def before(a, b):
        assert pos[a] < pos[b], (a, b)
    for u in range(n_units):
        c = u // 4
        before(('XQ', c), ('S', u)); before(('XO', c), ('P', u)); before(('XO', c), ('O', u))
        before(('S', u), ('O', u)); before(('O', u), ('V', u)); before(('O', u), ('Q', u)); before(('P', u), ('Q', u))
        before(('V', u), ('K', u)); before(('Q', u), ('K', u))
        before(('O', u), ('YO', c)); before(('Q', u), ('YQ', c))
        before(('YO', c), ('WO', 0)); before(('YQ', c), ('WQ', 0))
        for g, b0 in enumerate(kvsplit):
            if u // G >= b0:
                before(('WAIT', g + 1), ('S', u)); before(('WAIT', g + 1), ('P', u))
    return sched


def run_full(xa, ka, va, wqa, woa, xb, kb, vb, wqb, wob, go, order="P2 S0 O1 Q2 V1 K2",
             extra="XQ@-4/P XO@-3/P YO@6/P YQ@7/P", moves="XO0>XQ0 XQ1>S0 S1>XQ1 XO1>S1 YO7>P31 WO0>K31 YQ6>P30",
             kvsplit=(), waits="", morder=(2, 3, 0, 1, 4, 5, 6), show=False, ebf=1, cacc=0, yorder=(0, 3, 4, 6, 1, 2, 5), rchunk=32, nsteps=2 * NS):
    sched = build_sched(order, extra, moves, kvsplit, waits)
    if show:
        print(" ".join(f"{a}{b}" for a, b in sched))
    anyspec = pl.BlockSpec(memory_space=pl.ANY)
    sds = lambda s: jax.ShapeDtypeStruct(s, BF16)
    br_out = [sds((T, D)), sds(ka.shape), sds(va.shape), sds(wqa.shape), sds(woa.shape)]
    V = pltpu.VMEM
    scratch = ([V((2, B, G, SK, DH), BF16)] * 4
               + [V((2, D, W), BF16), V((2, W, D), BF16), V((2, D, W), BF16), V((2, W, D), BF16)]
               + [V((T, D), BF16)] * 2 + [V((2, T, D), BF16)] * 2
               + [V((16, TH, 128), BF16)] * 2 + [V((7, TH // 128, DHF, 128), BF16)] * 2
               + [V((7, TH, DP), F32), V((2, TH, DC), F32)] * 2
               + [V((2, 2, TH, DH), BF16)] * 2 + [V((9, TH, DH), BF16)] * 2 + [V((4, 4, SQ, 128), BF16)]
               + [pltpu.SemaphoreType.DMA((2, 4 + 2 * len(kvsplit))), pltpu.SemaphoreType.DMA((2, 4)),
                  pltpu.SemaphoreType.DMA((6,))])
    outs = pl.pallas_call(
        functools.partial(kernel, sched=sched, kvsplit=kvsplit, morder=morder, ebf=ebf, cacc=cacc, yorder=yorder, rchunk=rchunk, nsteps=nsteps),
        grid=(nsteps,),
        in_specs=[anyspec] * 11,
        out_specs=[anyspec] * 11,
        out_shape=[sds((T, 2 * D))] + br_out + br_out,
        scratch_shapes=scratch,
        compiler_params=pltpu.CompilerParams(dimension_semantics=("arbitrary",), vmem_limit_bytes=110 * 2**20,
                                             disable_bounds_checks=True),
        name=NAME,
    )(xa.reshape(T, D), ka, va, wqa, woa, xb.reshape(T, D), kb, vb, wqb, wob, go.reshape(T, 2 * D))
    o = list(outs)
    o[0] = o[0].reshape(B, SQ, 2 * D)
    o[1] = o[1].reshape(B, SQ, D)
    o[6] = o[6].reshape(B, SQ, D)
    return tuple(o)


@jax.jit
def pallas_concat_heads__gqa_block_cached__gqa_block_cached__near_ridge_kernel(
    A_x, A_k_cache, A_v_cache, A_wq, A_wo, B_x, B_k_cache, B_v_cache, B_wq, B_wo, grad_out
):
    return run_full(A_x, A_k_cache, A_v_cache, A_wq, A_wo, B_x, B_k_cache, B_v_cache, B_wq, B_wo,
                    grad_out)
```

```python
import contextlib
import functools

import jax
import jax.numpy as jnp
from jax import lax
from jax.experimental import pallas as pl
from jax.experimental.pallas import tpu as pltpu

NAME = "concat_heads_gqa_fwd_bwd"
B, SQ, D, H, SK, DH = 16, 112, 640, 32, 512, 128
T = B * SQ
TH = T // 2
G = 2
W = G * DH
NS = H // G
NB = B // 2
NK = TH // 128
ND = D // 128
DP = 256
DC = D - 2 * DP
DHF = D // 2
F32, BF16, U32 = jnp.float32, jnp.bfloat16, jnp.uint32
NN = (((1,), (0,)), ((), ()))
NT = (((1,), (1,)), ((), ()))
TN = (((0,), (0,)), ((), ()))
SCALE = DH ** -0.5
LOG2E = 1.4426950408889634
BORD = (0, 2, 6, 5, 3, 4, 1)


def dot(a, b, dims):
    return lax.dot_general(a, b, dims, preferred_element_type=F32)


def combos(z11, z12, z21, z22):
    f11, f12, f21, f22 = (z.astype(F32) for z in (z11, z12, z21, z22))
    return [c.astype(BF16) for c in
            (f11 + f22, f21 + f22, z11, z22, f11 + f12, f21 - f11, f12 - f22)]


def recombine(m):
    return (m[0] + m[3] - m[4] + m[6], m[2] + m[4], m[1] + m[3], m[0] - m[1] + m[2] + m[5])


def upk(x):
    return pltpu.bitcast(x, BF16)


def pk(x):
    return pltpu.bitcast(x, U32)


def wait_for(buf, sem):
    pltpu.make_async_copy(buf, buf, sem).wait()


def rows(start, size, align):
    return pl.ds(start if isinstance(start, int) else pl.multiple_of(start, align), size)


def kernel(xa, ka, va, wqa, woa, xb, kb, vb, wqb, wob, go,
           out, dxa, dka, dva, dwqa, dwoa, dxb, dkb, dvb, dwqb, dwob,
           kbuf, vbuf, dkbuf, dvbuf, wqbuf, wobuf, dwqbuf, dwobuf,
           xbuf, gobuf, obuf, dxbuf,
           xc, gc, xt, gt, om, ol, dm, dl, q_s, do_s, oc, dqc, eb_s,
           sem_in, sem_out, sem_act, sem_g, *, sched, sched0, morder, morder0, yorder, scopes):
    br = ((xa, ka, va, wqa, woa, dxa, dka, dva, dwqa, dwoa),
          (xb, kb, vb, wqb, wob, dxb, dkb, dvb, dwqb, dwob))
    scope = jax.named_scope if scopes else (lambda name: contextlib.nullcontext())
    nsteps = 2 * NS
    early = nsteps - 2

    k32, v32, q32, do32, oc32, dqc32, xc32, gc32, xt32, gt32, eb32 = (
        z.bitcast(U32) for z in (kbuf, vbuf, q_s, do_s, oc, dqc, xc, gc, xt, gt, eb_s))

    def start_w(rr, hp, s):
        wq, wo = br[rr][3:5]
        cols = rows(hp * W, W, W)
        pltpu.make_async_copy(wq.at[:, cols], wqbuf.at[s], sem_in.at[s, 0]).start()
        pltpu.make_async_copy(wo.at[cols, :], wobuf.at[s], sem_in.at[s, 1]).start()

    def start_in(rr, hp, s):
        k, v = br[rr][1:3]
        start_w(rr, hp, s)
        pltpu.make_async_copy(k.at[:, pl.ds(hp * G, G)], kbuf.at[s], sem_in.at[s, 2]).start()
        pltpu.make_async_copy(v.at[:, pl.ds(hp * G, G)], vbuf.at[s], sem_in.at[s, 3]).start()

    def kv_group(g, act):
        bs = pl.ds(2 * g, 2)
        for n, (src, dst) in enumerate(((ka, kbuf), (va, vbuf))):
            act(src.at[bs, pl.ds(0, G)], dst.at[0, bs], sem_g.at[g, n])

    def start_kv1(g):
        bs = pl.ds(2 * g, 2)
        for n, (src, dst) in enumerate(((ka, kbuf), (va, vbuf))):
            pltpu.make_async_copy(src.at[bs, pl.ds(G, G)], dst.at[1, bs], sem_in.at[1, 2 + n]).start()

    def x_group(g, act):
        rs = rows(2 * SQ * g, 2 * SQ, 16)
        act(xa.at[rs], xbuf.at[rs], sem_g.at[g, 2])
        act(go.at[rs, pl.ds(0, D)], gobuf.at[rs], sem_g.at[g, 3])

    start = lambda src, dst, sem: pltpu.make_async_copy(src, dst, sem).start()
    wait = lambda src, dst, sem: wait_for(dst, sem)

    def wait_out(s):
        for n, buf in enumerate((dkbuf, dvbuf, dwqbuf, dwobuf)):
            wait_for(buf.at[s], sem_out.at[s, n])

    def start_act_out(rr, which, rs, prio=0):
        dst, c0 = (out, rr * D) if which == 0 else (br[rr][5], 0)
        pltpu.make_async_copy((obuf, dxbuf)[which].at[rr, rs], dst.at[rs, pl.ds(c0, D)],
                              sem_act.at[2 + which]).start(priority=prio)

    def for_step(step, fn, lo=0, hi=nsteps):
        for rr in range(2):
            a, b = max(lo, rr * NS), min(hi, (rr + 1) * NS)
            if a < b:
                @pl.when(jnp.logical_and(step >= a, step < b))
                def _():
                    fn(rr, step - rr * NS)

    def natural(src, cmb, c32, be):
        for p in range(0, SQ, 32):
            n_r = min(32, SQ - p)
            r1, r2 = rows(2 * be * SQ + p, n_r, 16), rows((2 * be + 1) * SQ + p, n_r, 16)
            ro, rh = rows(be * SQ + p, n_r, 16), rows(be * (SQ // 2) + p // 2, n_r // 2, 8)
            for c in range(2):
                f = lambda rr, d: src[rr, pl.ds(d * DP + c * 128, 128)]
                cs = combos(f(r1, 0), f(r2, 0), f(r1, 1), f(r2, 1))
                for n in (0, 1, 4, 5, 6):
                    cmb[2 * n + c, ro, :] = cs[n]
                c32[4 + c, rh, :] = pk(f(r1, 0))
                c32[6 + c, rh, :] = pk(f(r2, 1))
            c32[14, rh, :] = pk(src[r1, pl.ds(2 * DP, DC)])
            c32[15, rh, :] = pk(src[r2, pl.ds(2 * DP, DC)])

    def transposed(src, cmt, c32, c):
        base = [((8 * c + g) // 7) * 2 * SQ + ((8 * c + g) % 7) * 16 for g in range(8)]
        tile_t = lambda t, d: jnp.concatenate(
            [src[rows(r0 + t * SQ, 16, 16), pl.ds(d * 128, 128)] for r0 in base], axis=0).T
        for d in range(ND):
            z1, z2 = tile_t(0, d), tile_t(1, d)
            cs = combos(z1[:64], z2[:64], z1[64:], z2[64:])
            for n in (0, 1, 4, 5, 6):
                cmt[n, c, pl.ds(d * 64, 64), :] = cs[n]
            c32[2, c, pl.ds(d * 32, 32), :] = pk(z1)[:32]
            c32[3, c, pl.ds(d * 32, 32), :] = pk(z2)[32:]

    def make_stages(i, slot, first, pair_of):
        st, ov, dqv, wts = {}, {}, {}, {}
        hrow = lambda be: rows(be * (SQ // 2), SQ // 2, 8)
        split = lambda u: (u // 4, (u // 2) % 2, u % 2)
        getk = lambda p, t, j: upk(k32[slot, 2 * pair_of(p) + t, j])
        getv = lambda p, t, j: upk(v32[slot, 2 * pair_of(p) + t, j])
        getq = lambda p, t, j: upk(q32[j, t, hrow(p), :])
        getdo = lambda p, t, j: upk(do32[j, t, hrow(p), :])
        tiles = lambda n: jnp.concatenate([upk(eb32[n, c]) for c in range(SK // 128)], axis=1)

        def store_tiles(n, val):
            for c in range(SK // 128):
                eb_s[n, c] = val[:, c * 128:(c + 1) * 128].astype(BF16)

        def weights(which):
            if not wts:
                wq, wo = wqbuf[slot], wobuf[slot]
                fq = lambda j, d: wq[d * DP:(d + 1) * DP, j * DH:(j + 1) * DH]
                fo = lambda j, d: wo[j * DH:(j + 1) * DH, d * DP:(d + 1) * DP]
                wts['q'] = combos(fq(0, 0), fq(0, 1), fq(1, 0), fq(1, 1)), wq[2 * DP:, :]
                wts['o'] = combos(fo(0, 0), fo(0, 1), fo(1, 0), fo(1, 1)), wo[:, 2 * DP:]
            return wts[which]

        def start_dkv(rr, hp, which, bs):
            src, dst = (dkbuf, dvbuf)[which], br[rr][6 + which]
            pltpu.make_async_copy(src.at[slot, bs], dst.at[bs, pl.ds(hp * G, G)], sem_out.at[slot, which]).start()

        def start_dw(rr, hp):
            dwq, dwo = br[rr][8:10]
            cols = rows(hp * W, W, W)
            pltpu.make_async_copy(dwqbuf.at[slot], dwq.at[:, cols], sem_out.at[slot, 2]).start()
            pltpu.make_async_copy(dwobuf.at[slot], dwo.at[cols, :], sem_out.at[slot, 3]).start()

        def proj_in(p, c32, which, dims, dst, mul):
            wc, wl = weights(which)
            get = lambda n: upk(c32[n, hrow(pair_of(p)), :])
            rest = [dot(get(14 + t), wl, dims) for t in range(2)]
            m = [None] * 7
            for n in (morder0 if first else morder):
                lhs = jnp.concatenate([get(2 * BORD[n]), get(2 * BORD[n] + 1)], axis=1)
                m[n] = dot(lhs, wc[n], dims)
            c = recombine(m)
            for t in range(2):
                for j in range(2):
                    val = c[2 * j + t] + rest[t][:, j * DH:(j + 1) * DH]
                    if mul is not None:
                        val = val * mul
                    dst[j, t, pl.ds(p * SQ, SQ), :] = val.astype(BF16)

        def proj_out(p, vals, cst, c32, which, dims, macc, lacc, stage):
            wc, wl = weights(which)
            be = pair_of(p)
            ro = rows(be * SQ, SQ, 16)
            z = [[vals.pop((p, t, j)) for j in range(2)] for t in range(2)]
            cs = combos(z[0][0], z[0][1], z[1][0], z[1][1]) + [z[0][1].astype(BF16), z[1][0].astype(BF16)]
            for n in range(9):
                cst[n, ro, :] = cs[n]
            get = lambda n: upk(c32[n, hrow(be), :])
            head = (lambda j: wl[j * DH:(j + 1) * DH, :]) if dims is NN else (lambda j: wl[:, j * DH:(j + 1) * DH])
            m = [None] * 7
            for n in yorder:
                m[n] = dot(get(n), wc[BORD[n]], dims)
                if not first:
                    m[n] = m[n] + macc[n, ro, :]
                macc[n, ro, :] = m[n]
            c = None if first else recombine(m)
            for t, (n0, n1) in enumerate(((2, 7), (8, 3))):
                rest = dot(get(n0), head(0), dims) + dot(get(n1), head(1), dims)
                if not first:
                    rest = rest + lacc[t, ro, :]
                lacc[t, ro, :] = rest
                if not first:
                    row = jnp.concatenate([c[2 * t], c[2 * t + 1], rest], axis=1)
                    stage[i // NS, pl.ds((2 * be + t) * SQ, SQ), :] = row.astype(BF16)
            if not first:
                @pl.when(i == nsteps - 1)
                def _():
                    start_act_out(1, 0 if which == 'o' else 1, pl.ds(2 * be * SQ, 2 * SQ))

        def proj_w(c32, zt32):
            m = [dot(jnp.concatenate([upk(zt32[n, c]) for c in range(NK)], axis=1), upk(c32[BORD[n]]), NN)
                 for n in range(7)]
            c = recombine(m)
            top = jnp.concatenate([c[0], c[1]], axis=1)
            bot = jnp.concatenate([c[2], c[3]], axis=1)
            rs = [z[d * 64:(d + 1) * 64] for d in range(ND) for z in (top, bot)]
            return jnp.concatenate(rs, axis=0).astype(BF16)

        def S(u):
            s = dot(getq(*split(u)), getk(*split(u)), NT)
            e = jnp.exp2(s - jnp.max(s, axis=-1, keepdims=True))
            l = jnp.sum(e, axis=-1, keepdims=True)
            rcp = pl.reciprocal(l, approx=True)
            st.setdefault(u, {})['r'] = rcp * (2.0 - l * rcp)
            store_tiles(u % 4, e)

        def P(u):
            st.setdefault(u, {})['dp'] = dot(getdo(*split(u)), getv(*split(u)), NT)

        def O(u):
            o = dot(tiles(u % 4), getv(*split(u)), NN) * st[u]['r']
            dof = getdo(*split(u)).astype(F32)
            st[u]['delta'] = jnp.sum(o * dof, axis=-1, keepdims=True)
            st[u]['dor'] = (dof * st[u]['r']).astype(BF16)
            ov[split(u)] = o

        def Q(u):
            ds = tiles(u % 4).astype(F32) * (st[u]['dp'] - st[u]['delta'])
            if first:
                store_tiles(4 + u % 4, ds)
                st[u]['ds'] = tiles(4 + u % 4)
            else:
                st[u]['ds'] = ds.astype(BF16)
            dqv[split(u)] = dot(st[u]['ds'], getk(*split(u)), NN) * (st[u]['r'] * SCALE)

        def tn_store(u, lhs, rhs, which):
            p, t, j = split(u)
            dst, b = (dkbuf, dvbuf)[which], 2 * pair_of(p) + t
            if first:
                for c in range(SK // 128):
                    res = dot(lhs[:, c * 128:(c + 1) * 128], rhs, TN)
                    dst[slot, b, j, pl.ds(c * 128, 128), :] = res.astype(BF16)
            else:
                dst[slot, b, j] = dot(lhs, rhs, TN).astype(BF16)
                if u % 4 == 3:
                    for_step(i, lambda rr, hp: start_dkv(rr, hp, which, pl.ds(2 * p, 2)), lo=early)

        def V(u):
            tn_store(u, tiles(u % 4), st[u]['dor'], 1)

        def K(u):
            qr = (getq(*split(u)).astype(F32) * (st[u]['r'] * (1.0 / LOG2E))).astype(BF16)
            tn_store(u, st[u]['ds'], qr, 0)

        def WO(_):
            dwobuf[slot] = proj_w(oc32, gt32).T

        def WQ(_):
            dwqbuf[slot] = proj_w(dqc32, xt32)

        def END(_):
            for which in range(2):
                for_step(i, lambda rr, hp: start_dkv(rr, hp, which, pl.ds(0, B)), hi=early)
            for_step(i + 2, lambda rr, hp: start_in(rr, hp, slot))
            for_step(i, start_dw)

        nxt = lambda p: jnp.minimum(pair_of(p) + 1, NB - 1)
        tile = lambda p: jnp.minimum(pair_of(p), NK - 1)
        return dict(
            S=S, P=P, O=O, V=V, Q=Q, K=K, WO=WO, WQ=WQ, END=END,
            XQ=lambda p: proj_in(p, xc32, 'q', NN, q_s, SCALE * LOG2E),
            XO=lambda p: proj_in(p, gc32, 'o', NT, do_s, None),
            YO=lambda p: proj_out(p, ov, oc, oc32, 'o', NN, om, ol, obuf),
            YQ=lambda p: proj_out(p, dqv, dqc, dqc32, 'q', NT, dm, dl, dxbuf),
            NX=lambda p: natural(xbuf, xc, xc32, nxt(p)),
            NG=lambda p: natural(gobuf, gc, gc32, nxt(p)),
            TX=lambda p: transposed(xbuf, xt, xt32, tile(p)),
            TG=lambda p: transposed(gobuf, gt, gt32, tile(p)))

    def first_step(i):
        @pl.when(i == 0)
        def _():
            x_group(0, wait)

        @pl.when(i == NS)
        def _():
            for which in range(2):
                start_act_out(0, which, pl.ds(0, T), prio=1)
            wait_for(xbuf, sem_act.at[0])
            wait_for(gobuf, sem_act.at[1])
            for n, buf in enumerate((kbuf, vbuf)):
                wait_for(buf.at[0], sem_in.at[0, 2 + n])
            wait_out(0)
        natural(xbuf, xc, xc32, 0)
        natural(gobuf, gc, gc32, 0)
        for n, buf in enumerate((wqbuf, wobuf)):
            wait_for(buf.at[0], sem_in.at[0, n])

        def pair(be, carry):
            with scope("pair"):
                @pl.when(i == 0)
                def _():
                    kv_group(be, wait)

                @pl.when(jnp.logical_and(i == 0, be + 1 < NB))
                def _():
                    x_group(be + 1, wait)

                @pl.when(jnp.logical_and(i == 0, be + 2 < NB))
                def _():
                    kv_group(be + 2, start)

                @pl.when(jnp.logical_and(i == 0, be + 3 < NB))
                def _():
                    x_group(be + 3, start)

                @pl.when(i == 0)
                def _():
                    start_kv1(be)
                fns = make_stages(i, 0, True, lambda p: be)
                for name, idx in sched0:
                    fns[name](idx)
            return carry
        lax.fori_loop(0, NB, pair, 0)

        @pl.when(i == 0)
        def _():
            pltpu.make_async_copy(xb, xbuf, sem_act.at[0]).start(priority=1)
            pltpu.make_async_copy(go.at[:, pl.ds(D, D)], gobuf, sem_act.at[1]).start(priority=1)
        fns = make_stages(i, 0, True, None)
        for name in ('WO', 'WQ', 'END'):
            fns[name](0)

    def regular_step(i, carry):
        with scope("reg"):
            slot = i % 2
            for n, buf in enumerate((wqbuf, wobuf, kbuf, vbuf)):
                wait_for(buf.at[slot], sem_in.at[slot, n])

            @pl.when(i >= 2)
            def _():
                wait_out(slot)
            fns = make_stages(i, slot, False, lambda p: p)
            for name, idx in sched:
                fns[name](idx)
        return carry

    def branch(rr, carry):
        with scope("first"):
            first_step(rr * NS)
        lax.fori_loop(rr * NS + 1, (rr + 1) * NS, regular_step, 0)
        return carry

    x_group(0, start)
    start_w(0, 0, 0)
    kv_group(0, start)
    x_group(1, start)
    kv_group(1, start)
    x_group(2, start)
    start_w(0, 1, 1)
    lax.fori_loop(0, 2, branch, 0)
    with scope("epi"):
        wait_out(0)
        wait_out(1)
        wait_for(obuf, sem_act.at[2])
        wait_for(dxbuf, sem_act.at[3])


def parse(z):
    name = z.rstrip('0123456789')
    return name, int(z[len(name):])


def check(sched, n_units):
    pos = {it: n for n, it in enumerate(sched)}
    assert len(pos) == len(sched)
    for u in range(n_units):
        p = u // 4
        deps = [(('XQ', p), ('S', u)), (('XO', p), ('P', u)), (('XO', p), ('O', u)), (('S', u), ('O', u)),
                (('O', u), ('V', u)), (('O', u), ('Q', u)), (('P', u), ('Q', u)), (('Q', u), ('K', u)),
                (('O', u), ('YO', p)), (('Q', u), ('YQ', p))]
        if n_units > 4:
            deps += [(('YO', p), ('WO', 0)), (('YQ', p), ('WQ', 0))]
        else:
            deps += [(('XQ', 0), ('NX', 0)), (('XO', 0), ('NG', 0))]
        if u + 4 < n_units:
            deps += [(('V', u), ('S', u + 4)), (('Q', u), ('S', u + 4))]
        for a, b in deps:
            assert pos[a] < pos[b], (a, b)


def build_sched(order, extra, moves):
    order = [(w[0], int(w[1:])) for w in order.split()]
    n_units = G * B
    ex = []
    for w in extra.split():
        name, rest = w.split('@')
        off, after = rest.split('/')
        ex.append((name, int(off), after))
    sched = []
    for t in range(-16, n_units + 16):
        for nm, lag in order:
            if 0 <= t - lag < n_units:
                sched.append((nm, t - lag))
            for en, off, after in ex:
                if after == nm and (t - off) % 4 == 0 and 0 <= (t - off) // 4 < NB:
                    sched.append((en, (t - off) // 4))
    sched += [('WO', 0), ('WQ', 0), ('END', 0)]
    for mv in moves.split():
        a, b = map(parse, mv.split('>'))
        sched.remove(a)
        sched.insert(sched.index(b) + 1, a)
    assert len(sched) == 6 * n_units + 4 * NB + 3
    check(sched, n_units)
    return sched


def run_full(xa, ka, va, wqa, woa, xb, kb, vb, wqb, wob, go, order="P2 S0 O1 Q2 V1 K2",
             extra="XQ@-4/V XO@-3/V YO@6/V YQ@7/V",
             moves="XO0>XQ0 XQ1>S0 S1>XQ1 XO1>S1 XQ2>P0 YO7>P31 WO0>K31 YQ6>P30 YQ5>P26 YO6>P27",
             first="XQ0 XO0 TX0 S0 S1 P0 S2 P1 O0 NX0 S3 O1 V0 Q0 V1 K0 TG0 P2 O2 Q1 V2 K1 NG0 P3 O3 Q2 V3 K2 Q3 YO0 K3 YQ0",
             morder=(2, 3, 0, 1, 4, 5, 6), morder0=(1, 4, 0, 2, 3, 5, 6), yorder=(0, 3, 4, 6, 1, 2, 5),
             scopes=False, semchk=False, pads=()):
    sched = build_sched(order, extra, moves)
    sched0 = [parse(z) for z in first.split()]
    check(sched0, 4)
    anyspec = pl.BlockSpec(memory_space=pl.ANY)
    sds = lambda s: jax.ShapeDtypeStruct(s, BF16)
    br_out = [sds((T, D)), sds(ka.shape), sds(va.shape), sds(wqa.shape), sds(woa.shape)]
    V = pltpu.VMEM
    scratch = ([V((2, B, G, SK, DH), BF16)] * 4
               + [V((2, D, W), BF16), V((2, W, D), BF16), V((2, D, W), BF16), V((2, W, D), BF16)]
               + [V((T, D), BF16)] * 2 + [V((2, T, D), BF16)] * 2
               + [V((16, TH, 128), BF16)] * 2 + [V((7, NK, DHF, 128), BF16)] * 2
               + [V((7, TH, DP), F32), V((2, TH, DC), F32)] * 2
               + [V((2, 2, TH, DH), BF16)] * 2 + [V((9, TH, DH), BF16)] * 2
               + [V((8, SK // 128, SQ, 128), BF16)]
               + [pltpu.SemaphoreType.DMA((2, 4)), pltpu.SemaphoreType.DMA((2, 4)),
                  pltpu.SemaphoreType.DMA((4,)), pltpu.SemaphoreType.DMA((NB, 4))])
    kern0 = functools.partial(kernel, sched=sched, sched0=sched0, morder=morder, morder0=morder0, yorder=yorder,
                              scopes=scopes)
    pads = dict(pads)
    keep = []
    sc2 = []
    for n, z in enumerate(scratch):
        if n in pads:
            sc2.append(V((pads[n], 128), F32))
        keep.append(22 + len(sc2))
        sc2.append(z)
    scratch = sc2
    def kern(*refs):
        for n, z in enumerate(refs[22:]):
            if 22 + n not in keep:
                z[0:8, :] = jnp.zeros((8, 128), F32)
        kern0(*refs[:22], *[refs[k] for k in keep])
    outs = pl.pallas_call(
        kern,
        in_specs=[anyspec] * 11,
        out_specs=[anyspec] * 11,
        out_shape=[sds((T, 2 * D))] + br_out + br_out,
        scratch_shapes=scratch,
        compiler_params=pltpu.CompilerParams(vmem_limit_bytes=100 * 2**20, disable_bounds_checks=True,
                                             disable_semaphore_checks=not semchk),
        name=NAME,
    )(xa.reshape(T, D), ka, va, wqa, woa, xb.reshape(T, D), kb, vb, wqb, wob, go.reshape(T, 2 * D))
    o = list(outs)
    o[0] = o[0].reshape(B, SQ, 2 * D)
    o[1] = o[1].reshape(B, SQ, D)
    o[6] = o[6].reshape(B, SQ, D)
    return tuple(o)


@jax.jit
def pallas_concat_heads__gqa_block_cached__gqa_block_cached__near_ridge_kernel(
    A_x, A_k_cache, A_v_cache, A_wq, A_wo, B_x, B_k_cache, B_v_cache, B_wq, B_wo, grad_out
):
    return run_full(A_x, A_k_cache, A_v_cache, A_wq, A_wo, B_x, B_k_cache, B_v_cache, B_wq, B_wo,
                    grad_out)
```

```python
import jax
import jax.numpy as jnp
from jax import lax
from jax.experimental import pallas as pl
from jax.experimental.pallas import tpu as pltpu

NAME = "concat_heads_gqa_fwd_bwd"
B, SQ, D, H, SK, DH = 16, 112, 640, 32, 512, 128
T = B * SQ
TH = T // 2
G = 2
W = G * DH
NS = H // G
NSTEPS = 2 * NS
EARLY = NSTEPS - 2
NB = B // 2
NK = TH // 128
ND = D // 128
NC = SK // 128
DP = 256
DC = D - 2 * DP
DHF = D // 2
F32, BF16, U32 = jnp.float32, jnp.bfloat16, jnp.uint32
NN = (((1,), (0,)), ((), ()))
NT = (((1,), (1,)), ((), ()))
TN = (((0,), (0,)), ((), ()))
SCALE = DH ** -0.5
LOG2E = 1.4426950408889634
BORD = (0, 2, 6, 5, 3, 4, 1)


def combos(z11, z12, z21, z22):
    f11, f12, f21, f22 = (z.astype(F32) for z in (z11, z12, z21, z22))
    return [c.astype(BF16) for c in
            (f11 + f22, f21 + f22, z11, z22, f11 + f12, f21 - f11, f12 - f22)]


def recombine(m):
    return (m[0] + m[3] - m[4] + m[6], m[2] + m[4], m[1] + m[3], m[0] - m[1] + m[2] + m[5])


def dot(a, b, dims):
    return lax.dot_general(a, b, dims, preferred_element_type=F32)


def upk(x):
    return pltpu.bitcast(x, BF16)


def pk(x):
    return pltpu.bitcast(x, U32)


def rows(start, size, align):
    return pl.ds(start if isinstance(start, int) else pl.multiple_of(start, align), size)


def start(src, dst, sem, priority=0):
    pltpu.make_async_copy(src, dst, sem).start(priority=priority)


def wait_for(buf, sem):
    pltpu.make_async_copy(buf, buf, sem).wait()


def parse(items):
    out = []
    for z in items.split():
        name = z.rstrip('0123456789')
        out.append((name, int(z[len(name):])))
    return out


def regular_schedule():
    n_units = G * B
    sched = []
    for t in range(-4, n_units + 8):
        for name, lag in parse("P2 S0 O1 Q2 V1 K2"):
            if 0 <= t - lag < n_units:
                sched.append((name, t - lag))
            if name == 'V':
                for pair_stage, offset in (('XQ', -4), ('XO', -3), ('YO', 6), ('YQ', 7)):
                    if (t - offset) % 4 == 0 and 0 <= (t - offset) // 4 < NB:
                        sched.append((pair_stage, (t - offset) // 4))
    sched += parse("WO0 WQ0 END0")
    for move in ("XQ1 S0", "S1 XQ1", "XO1 S1", "XQ2 P0", "YO7 P31", "WO0 K31", "YQ6 P30", "YQ5 P26", "YO6 P27"):
        a, b = parse(move)
        sched.remove(a)
        sched.insert(sched.index(b) + 1, a)
    return sched


def check(sched, n_units):
    pos = {it: n for n, it in enumerate(sched)}
    assert len(pos) == len(sched)
    for u in range(n_units):
        p = u // 4
        deps = [(('XQ', p), ('S', u)), (('XO', p), ('S', u)), (('XO', p), ('P', u)), (('S', u), ('O', u)),
                (('S', u), ('V', u)), (('O', u), ('Q', u)), (('P', u), ('Q', u)), (('Q', u), ('K', u)),
                (('O', u), ('YO', p)), (('Q', u), ('YQ', p))]
        if n_units > 4:
            deps += [(('YO', p), ('WO', 0)), (('YQ', p), ('WQ', 0))]
        else:
            deps += [(('XQ', 0), ('NX', 0)), (('XO', 0), ('NG', 0))]
        if u + 4 < n_units:
            deps += [(('V', u), ('S', u + 4)), (('Q', u), ('S', u + 4))]
        for a, b in deps:
            assert pos[a] < pos[b], (a, b)
    return sched


SCHED = check(regular_schedule(), G * B)
SCHED_PAIR = check(parse("XQ0 XO0 TX0 S0 S1 S2 P0 O0 S3 P1 O1 NX0 V0 Q0 P2 O2 K0 V1 Q1 P3 O3 K1 TG0 "
                         "V2 Q2 V3 Q3 K2 NG0 YO0 K3 YQ0"), 4)


def kernel(xa, ka, va, wqa, woa, xb, kb, vb, wqb, wob, go,
           out, dxa, dka, dva, dwqa, dwoa, dxb, dkb, dvb, dwqb, dwob,
           kbuf, vbuf, dkbuf, dvbuf, wqbuf, wobuf, dwqbuf, dwobuf,
           xbuf, gobuf, obuf, dxbuf,
           xc, gc, xt, gt, om, ol, dm, dl, q_s, do_s, oc, dqc, e_s,
           sem_in, sem_out, sem_act, sem_g):
    br = ((xa, ka, va, wqa, woa, dxa, dka, dva, dwqa, dwoa),
          (xb, kb, vb, wqb, wob, dxb, dkb, dvb, dwqb, dwob))
    k32, v32, q32, do32, oc32, dqc32, xc32, gc32, xt32, gt32, e32 = (
        z.bitcast(U32) for z in (kbuf, vbuf, q_s, do_s, oc, dqc, xc, gc, xt, gt, e_s))

    def start_w(rr, hp, s):
        wq, wo = br[rr][3:5]
        cols = rows(hp * W, W, W)
        start(wq.at[:, cols], wqbuf.at[s], sem_in.at[s, 0])
        start(wo.at[cols, :], wobuf.at[s], sem_in.at[s, 1])

    def start_in(rr, hp, s):
        k, v = br[rr][1:3]
        start_w(rr, hp, s)
        start(k.at[:, pl.ds(hp * G, G)], kbuf.at[s], sem_in.at[s, 2])
        start(v.at[:, pl.ds(hp * G, G)], vbuf.at[s], sem_in.at[s, 3])

    def wait_out(s):
        for n, buf in enumerate((dkbuf, dvbuf, dwqbuf, dwobuf)):
            wait_for(buf.at[s], sem_out.at[s, n])

    def start_act_out(rr, which, rs, priority=0):
        dst, c0 = (out, rr * D) if which == 0 else (br[rr][5], 0)
        start((obuf, dxbuf)[which].at[rr, rs], dst.at[rs, pl.ds(c0, D)], sem_act.at[2 + which], priority)

    def kv_group(g, act):
        bs = pl.ds(2 * g, 2)
        act(ka.at[bs, pl.ds(0, G)], kbuf.at[0, bs], sem_g.at[g, 0])
        act(va.at[bs, pl.ds(0, G)], vbuf.at[0, bs], sem_g.at[g, 1])

    def x_group(g, act):
        rs = rows(2 * SQ * g, 2 * SQ, 16)
        act(xa.at[rs], xbuf.at[rs], sem_g.at[g, 2])
        act(go.at[rs, pl.ds(0, D)], gobuf.at[rs], sem_g.at[g, 3])

    def start_kv_step1(g):
        bs = pl.ds(2 * g, 2)
        start(ka.at[bs, pl.ds(G, G)], kbuf.at[1, bs], sem_in.at[1, 2])
        start(va.at[bs, pl.ds(G, G)], vbuf.at[1, bs], sem_in.at[1, 3])

    wait = lambda src, dst, sem: wait_for(dst, sem)

    def for_step(step, fn, lo=0, hi=NSTEPS):
        for rr in range(2):
            a, b = max(lo, rr * NS), min(hi, (rr + 1) * NS)
            if a < b:
                @pl.when(jnp.logical_and(step >= a, step < b))
                def _():
                    fn(rr, step - rr * NS)

    def natural(src, cmb, c32, be):
        for p in range(0, SQ, 32):
            n_r = min(32, SQ - p)
            r1, r2 = rows(2 * be * SQ + p, n_r, 16), rows((2 * be + 1) * SQ + p, n_r, 16)
            ro, rh = rows(be * SQ + p, n_r, 16), rows(be * (SQ // 2) + p // 2, n_r // 2, 8)
            for c in range(2):
                f = lambda rr, d: src[rr, pl.ds(d * DP + c * 128, 128)]
                cs = combos(f(r1, 0), f(r2, 0), f(r1, 1), f(r2, 1))
                for n in (0, 1, 4, 5, 6):
                    cmb[2 * n + c, ro, :] = cs[n]
                c32[4 + c, rh, :] = pk(f(r1, 0))
                c32[6 + c, rh, :] = pk(f(r2, 1))
            c32[14, rh, :] = pk(src[r1, pl.ds(2 * DP, DC)])
            c32[15, rh, :] = pk(src[r2, pl.ds(2 * DP, DC)])

    def transposed(src, cmt, c32, c):
        base = [((8 * c + g) // 7) * 2 * SQ + ((8 * c + g) % 7) * 16 for g in range(8)]
        tile_t = lambda t, d: jnp.concatenate(
            [src[rows(r0 + t * SQ, 16, 16), pl.ds(d * 128, 128)] for r0 in base], axis=0).T
        for d in range(ND):
            z1, z2 = tile_t(0, d), tile_t(1, d)
            cs = combos(z1[:64], z2[:64], z1[64:], z2[64:])
            for n in (0, 1, 4, 5, 6):
                cmt[n, c, pl.ds(d * 64, 64), :] = cs[n]
            c32[2, c, pl.ds(d * 32, 32), :] = pk(z1)[:32]
            c32[3, c, pl.ds(d * 32, 32), :] = pk(z2)[32:]

    def make_stages(i, slot, first, pair_of):
        st, ov, dqv, wts = {}, {}, {}, {}
        hrow = lambda be: rows(be * (SQ // 2), SQ // 2, 8)
        split = lambda u: (u // 4, (u // 2) % 2, u % 2)
        getk = lambda p, t, j: upk(k32[slot, 2 * pair_of(p) + t, j])
        getv = lambda p, t, j: upk(v32[slot, 2 * pair_of(p) + t, j])
        getq = lambda p, t, j: upk(q32[j, t, hrow(p), :])
        getdo = lambda p, t, j: upk(do32[j, t, hrow(p), :])
        tiles = lambda n: jnp.concatenate([upk(e32[n, c]) for c in range(NC)], axis=1)

        def store_tiles(n, val):
            for c in range(NC):
                e_s[n, c] = val[:, c * 128:(c + 1) * 128].astype(BF16)

        def weights(which):
            if not wts:
                wq, wo = wqbuf[slot], wobuf[slot]
                fq = lambda j, d: wq[d * DP:(d + 1) * DP, j * DH:(j + 1) * DH]
                fo = lambda j, d: wo[j * DH:(j + 1) * DH, d * DP:(d + 1) * DP]
                wts['q'] = combos(fq(0, 0), fq(0, 1), fq(1, 0), fq(1, 1)), wq[2 * DP:, :]
                wts['o'] = combos(fo(0, 0), fo(0, 1), fo(1, 0), fo(1, 1)), wo[:, 2 * DP:]
            return wts[which]

        def start_dkv(rr, hp, which, bs):
            src, dst = (dkbuf, dvbuf)[which], br[rr][6 + which]
            start(src.at[slot, bs], dst.at[bs, pl.ds(hp * G, G)], sem_out.at[slot, which])

        def start_dw(rr, hp):
            dwq, dwo = br[rr][8:10]
            cols = rows(hp * W, W, W)
            start(dwqbuf.at[slot], dwq.at[:, cols], sem_out.at[slot, 2])
            start(dwobuf.at[slot], dwo.at[cols, :], sem_out.at[slot, 3])

        def proj_in(p, c32, which, dims, dst, mul):
            wc, wl = weights(which)
            get = lambda n: upk(c32[n, hrow(pair_of(p)), :])
            rest = [dot(get(14 + t), wl, dims) for t in range(2)]
            m = [None] * 7
            for n in ((1, 4, 0, 2, 3, 5, 6) if first else (2, 3, 0, 1, 4, 5, 6)):
                lhs = jnp.concatenate([get(2 * BORD[n]), get(2 * BORD[n] + 1)], axis=1)
                m[n] = dot(lhs, wc[n], dims)
            c = recombine(m)
            for t in range(2):
                for j in range(2):
                    val = c[2 * j + t] + rest[t][:, j * DH:(j + 1) * DH]
                    if mul is not None:
                        val = val * mul
                    dst[j, t, pl.ds(p * SQ, SQ), :] = val.astype(BF16)

        def proj_out(p, vals, cst, c32, which, dims, macc, lacc, stage):
            wc, wl = weights(which)
            be = pair_of(p)
            ro = rows(be * SQ, SQ, 16)
            z = [[vals.pop((p, t, j)) for j in range(2)] for t in range(2)]
            cs = combos(z[0][0], z[0][1], z[1][0], z[1][1]) + [z[0][1].astype(BF16), z[1][0].astype(BF16)]
            for n in range(9):
                cst[n, ro, :] = cs[n]
            get = lambda n: upk(c32[n, hrow(be), :])
            head = (lambda j: wl[j * DH:(j + 1) * DH, :]) if dims is NN else (lambda j: wl[:, j * DH:(j + 1) * DH])
            m = [None] * 7
            for n in (0, 3, 4, 6, 1, 2, 5):
                m[n] = dot(get(n), wc[BORD[n]], dims)
                if not first:
                    m[n] = m[n] + macc[n, ro, :]
                macc[n, ro, :] = m[n]
            c = None if first else recombine(m)
            for t, (n0, n1) in enumerate(((2, 7), (8, 3))):
                rest = dot(get(n0), head(0), dims) + dot(get(n1), head(1), dims)
                if not first:
                    rest = rest + lacc[t, ro, :]
                lacc[t, ro, :] = rest
                if not first:
                    row = jnp.concatenate([c[2 * t], c[2 * t + 1], rest], axis=1)
                    stage[i // NS, pl.ds((2 * be + t) * SQ, SQ), :] = row.astype(BF16)
            if not first:
                @pl.when(i == NSTEPS - 1)
                def _():
                    start_act_out(1, 0 if which == 'o' else 1, pl.ds(2 * be * SQ, 2 * SQ))

        def proj_w(c32, zt32):
            m = [dot(jnp.concatenate([upk(zt32[n, c]) for c in range(NK)], axis=1), upk(c32[BORD[n]]), NN)
                 for n in range(7)]
            c = recombine(m)
            top = jnp.concatenate([c[0], c[1]], axis=1)
            bot = jnp.concatenate([c[2], c[3]], axis=1)
            rs = [z[d * 64:(d + 1) * 64] for d in range(ND) for z in (top, bot)]
            return jnp.concatenate(rs, axis=0).astype(BF16)

        def S(u):
            s = dot(getq(*split(u)), getk(*split(u)), NT)
            e = jnp.exp2(s - jnp.max(s, axis=-1, keepdims=True))
            l = jnp.sum(e, axis=-1, keepdims=True)
            rcp = pl.reciprocal(l, approx=True)
            r = rcp * (2.0 - l * rcp)
            store_tiles(u % 4, e)
            st.setdefault(u, {}).update(r=r, dor=(getdo(*split(u)).astype(F32) * r).astype(BF16))

        def P(u):
            st.setdefault(u, {})['dp'] = dot(getdo(*split(u)), getv(*split(u)), NT)

        def O(u):
            o = dot(tiles(u % 4), getv(*split(u)), NN) * st[u]['r']
            st[u]['delta'] = jnp.sum(o * getdo(*split(u)).astype(F32), axis=-1, keepdims=True)
            ov[split(u)] = o

        def Q(u):
            ds = tiles(u % 4).astype(F32) * (st[u]['dp'] - st[u]['delta'])
            if first:
                store_tiles(4 + u % 4, ds)
                st[u]['ds'] = tiles(4 + u % 4)
            else:
                st[u]['ds'] = ds.astype(BF16)
            dqv[split(u)] = dot(st[u]['ds'], getk(*split(u)), NN) * (st[u]['r'] * SCALE)

        def kv_grad(u, lhs, rhs, which):
            p, t, j = split(u)
            dst, b = (dkbuf, dvbuf)[which], 2 * pair_of(p) + t
            if first:
                for c in range(NC):
                    dst[slot, b, j, pl.ds(c * 128, 128), :] = dot(lhs[:, c * 128:(c + 1) * 128], rhs, TN).astype(BF16)
            else:
                dst[slot, b, j] = dot(lhs, rhs, TN).astype(BF16)
                if u % 4 == 3:
                    for_step(i, lambda rr, hp: start_dkv(rr, hp, which, pl.ds(2 * p, 2)), lo=EARLY)

        def V(u):
            kv_grad(u, tiles(u % 4), st[u]['dor'], 1)

        def K(u):
            qr = (getq(*split(u)).astype(F32) * (st[u]['r'] * (1.0 / LOG2E))).astype(BF16)
            kv_grad(u, st[u]['ds'], qr, 0)

        def WO(_):
            dwobuf[slot] = proj_w(oc32, gt32).T

        def WQ(_):
            dwqbuf[slot] = proj_w(dqc32, xt32)

        def END(_):
            for which in range(2):
                for_step(i, lambda rr, hp: start_dkv(rr, hp, which, pl.ds(0, B)), hi=EARLY)
            for_step(i + 2, lambda rr, hp: start_in(rr, hp, slot))
            for_step(i, start_dw)

        nxt = lambda p: jnp.minimum(pair_of(p) + 1, NB - 1)
        tile = lambda p: jnp.minimum(pair_of(p), NK - 1)
        return dict(
            S=S, P=P, O=O, V=V, Q=Q, K=K, WO=WO, WQ=WQ, END=END,
            XQ=lambda p: proj_in(p, xc32, 'q', NN, q_s, SCALE * LOG2E),
            XO=lambda p: proj_in(p, gc32, 'o', NT, do_s, None),
            YO=lambda p: proj_out(p, ov, oc, oc32, 'o', NN, om, ol, obuf),
            YQ=lambda p: proj_out(p, dqv, dqc, dqc32, 'q', NT, dm, dl, dxbuf),
            NX=lambda p: natural(xbuf, xc, xc32, nxt(p)),
            NG=lambda p: natural(gobuf, gc, gc32, nxt(p)),
            TX=lambda p: transposed(xbuf, xt, xt32, tile(p)),
            TG=lambda p: transposed(gobuf, gt, gt32, tile(p)))

    def first_step(i):
        @pl.when(i == 0)
        def _():
            x_group(0, wait)

        @pl.when(i == NS)
        def _():
            for which in range(2):
                start_act_out(0, which, pl.ds(0, T), priority=1)
            wait_for(xbuf, sem_act.at[0])
            wait_for(gobuf, sem_act.at[1])
            wait_for(kbuf.at[0], sem_in.at[0, 2])
            wait_for(vbuf.at[0], sem_in.at[0, 3])
            wait_out(0)
        natural(xbuf, xc, xc32, 0)
        natural(gobuf, gc, gc32, 0)
        wait_for(wqbuf.at[0], sem_in.at[0, 0])
        wait_for(wobuf.at[0], sem_in.at[0, 1])

        def pair(be, carry):
            @pl.when(i == 0)
            def _():
                kv_group(be, wait)

            @pl.when(jnp.logical_and(i == 0, be + 1 < NB))
            def _():
                x_group(be + 1, wait)

            @pl.when(jnp.logical_and(i == 0, be + 2 < NB))
            def _():
                kv_group(be + 2, start)

            @pl.when(jnp.logical_and(i == 0, be + 3 < NB))
            def _():
                x_group(be + 3, start)

            @pl.when(i == 0)
            def _():
                start_kv_step1(be)
            stages = make_stages(i, 0, True, lambda p: be)
            for name, idx in SCHED_PAIR:
                stages[name](idx)
            return carry
        lax.fori_loop(0, NB, pair, 0)

        stages = make_stages(i, 0, True, None)
        stages['WO'](0)
        stages['WQ'](0)

        @pl.when(i == 0)
        def _():
            start(xb, xbuf, sem_act.at[0], priority=1)
            start(go.at[:, pl.ds(D, D)], gobuf, sem_act.at[1], priority=1)
        stages['END'](0)

    def regular_step(i):
        slot = i % 2
        for n, buf in enumerate((wqbuf, wobuf, kbuf, vbuf)):
            wait_for(buf.at[slot], sem_in.at[slot, n])

        @pl.when(i >= 2)
        def _():
            wait_out(slot)
        stages = make_stages(i, slot, False, lambda p: p)
        for name, idx in SCHED:
            stages[name](idx)

    def branch(rr, carry):
        first_step(rr * NS)

        def body(j, c):
            regular_step(rr * NS + j)
            return c
        lax.fori_loop(1, NS, body, 0)
        return carry

    x_group(0, start)
    start_w(0, 0, 0)
    kv_group(0, start)
    x_group(1, start)
    kv_group(1, start)
    x_group(2, start)
    start_w(0, 1, 1)
    lax.fori_loop(0, 2, branch, 0)
    wait_out(0)
    wait_out(1)
    wait_for(obuf, sem_act.at[2])
    wait_for(dxbuf, sem_act.at[3])


def run_full(A_x, A_k_cache, A_v_cache, A_wq, A_wo, B_x, B_k_cache, B_v_cache, B_wq, B_wo, grad_out):
    hbm = pl.BlockSpec(memory_space=pl.ANY)
    sds = lambda *s: jax.ShapeDtypeStruct(s, BF16)
    grads = [sds(T, D), sds(B, H, SK, DH), sds(B, H, SK, DH), sds(D, H * DH), sds(H * DH, D)]
    vmem = pltpu.VMEM
    scratch = (
        [vmem((2, B, G, SK, DH), BF16)] * 4
        + [vmem((2, D, W), BF16), vmem((2, W, D), BF16)] * 2
        + [vmem((T, D), BF16)] * 2 + [vmem((2, T, D), BF16)] * 2
        + [vmem((16, TH, 128), BF16)] * 2 + [vmem((7, NK, DHF, 128), BF16)] * 2
        + [vmem((7, TH, DP), F32), vmem((2, TH, DC), F32)] * 2
        + [vmem((2, 2, TH, DH), BF16)] * 2 + [vmem((9, TH, DH), BF16)] * 2
        + [vmem((8, NC, SQ, 128), BF16)]
        + [pltpu.SemaphoreType.DMA((2, 4)), pltpu.SemaphoreType.DMA((2, 4)),
           pltpu.SemaphoreType.DMA((4,)), pltpu.SemaphoreType.DMA((NB, 4))])
    outs = list(pl.pallas_call(
        kernel,
        in_specs=[hbm] * 11,
        out_specs=[hbm] * 11,
        out_shape=[sds(T, 2 * D)] + grads + grads,
        scratch_shapes=scratch,
        compiler_params=pltpu.CompilerParams(vmem_limit_bytes=100 * 2**20, disable_bounds_checks=True,
                                             disable_semaphore_checks=True),
        name=NAME,
    )(A_x.reshape(T, D), A_k_cache, A_v_cache, A_wq, A_wo,
      B_x.reshape(T, D), B_k_cache, B_v_cache, B_wq, B_wo, grad_out.reshape(T, 2 * D)))
    outs[0] = outs[0].reshape(B, SQ, 2 * D)
    outs[1] = outs[1].reshape(B, SQ, D)
    outs[6] = outs[6].reshape(B, SQ, D)
    return tuple(outs)


@jax.jit
def pallas_concat_heads__gqa_block_cached__gqa_block_cached__near_ridge_kernel(
    A_x: jax.Array,
    A_k_cache: jax.Array,
    A_v_cache: jax.Array,
    A_wq: jax.Array,
    A_wo: jax.Array,
    B_x: jax.Array,
    B_k_cache: jax.Array,
    B_v_cache: jax.Array,
    B_wq: jax.Array,
    B_wo: jax.Array,
    grad_out: jax.Array,
):
    return run_full(A_x, A_k_cache, A_v_cache, A_wq, A_wo, B_x, B_k_cache, B_v_cache, B_wq, B_wo, grad_out)
```

```python
import jax
import jax.numpy as jnp
from jax import lax
from jax.experimental import pallas as pl
from jax.experimental.pallas import tpu as pltpu

NAME = "concat_heads_gqa_fwd_bwd"
B, SQ, D, H, SK, DH = 16, 112, 640, 32, 512, 128
T = B * SQ
TH = T // 2
G = 2
W = G * DH
NS = H // G
NSTEPS = 2 * NS
EARLY = NSTEPS - 2
NB = B // 2
NK = TH // 128
ND = D // 128
NC = SK // 128
DP = 256
DC = D - 2 * DP
DHF = D // 2
F32, BF16 = jnp.float32, jnp.bfloat16
NN = (((1,), (0,)), ((), ()))
NT = (((1,), (1,)), ((), ()))
TN = (((0,), (0,)), ((), ()))
SCALE = DH ** -0.5
LOG2E = 1.4426950408889634
BORD = (0, 2, 6, 5, 3, 4, 1)


def combos(z11, z12, z21, z22, repack=False):
    f11, f12, f21, f22 = (z.astype(F32) for z in (z11, z12, z21, z22))
    if repack:
        z11, z22 = f11 + 0.0, f22 + 0.0
    return [c.astype(BF16) for c in
            (f11 + f22, f21 + f22, z11, z22, f11 + f12, f21 - f11, f12 - f22)]


def recombine(m):
    return (m[0] + m[3] - m[4] + m[6], m[2] + m[4], m[1] + m[3], m[0] - m[1] + m[2] + m[5])


def dot(a, b, dims):
    return lax.dot_general(a, b, dims, preferred_element_type=F32)


def rows(start, size, align):
    return pl.ds(start if isinstance(start, int) else pl.multiple_of(start, align), size)


def start(src, dst, sem, priority=0):
    pltpu.make_async_copy(src, dst, sem).start(priority=priority)


def wait_for(buf, sem):
    pltpu.make_async_copy(buf, buf, sem).wait()


def parse(items):
    out = []
    for z in items.split():
        name = z.rstrip('0123456789')
        out.append((name, int(z[len(name):])))
    return out


def regular_schedule():
    n_units = G * B
    sched = []
    for t in range(-4, n_units + 8):
        for name, lag in parse("P2 S0 O1 Q2 V1 K2"):
            if 0 <= t - lag < n_units:
                sched.append((name, t - lag))
            if name == 'V':
                for pair_stage, offset in (('XQ', -4), ('XO', -3), ('YO', 6), ('YQ', 7)):
                    if (t - offset) % 4 == 0 and 0 <= (t - offset) // 4 < NB:
                        sched.append((pair_stage, (t - offset) // 4))
    sched += parse("WO0 WQ0 END0")
    for move in ("XQ1 S0", "S1 XQ1", "XO1 S1", "XQ2 P0", "YO7 P31", "WO0 K31", "YQ6 P30", "YQ5 P26", "YO6 P27"):
        a, b = parse(move)
        sched.remove(a)
        sched.insert(sched.index(b) + 1, a)
    return sched


def check(sched, n_units):
    pos = {it: n for n, it in enumerate(sched)}
    assert len(pos) == len(sched)
    for u in range(n_units):
        p = u // 4
        deps = [(('XQ', p), ('S', u)), (('XO', p), ('S', u)), (('XO', p), ('P', u)), (('S', u), ('O', u)),
                (('S', u), ('V', u)), (('O', u), ('Q', u)), (('P', u), ('Q', u)), (('Q', u), ('K', u)),
                (('O', u), ('YO', p)), (('Q', u), ('YQ', p))]
        if n_units > 4:
            deps += [(('YO', p), ('WO', 0)), (('YQ', p), ('WQ', 0))]
        else:
            deps += [(('XQ', 0), ('NX', 0)), (('XO', 0), ('NG', 0))]
        if u + 4 < n_units:
            deps += [(('V', u), ('S', u + 4)), (('Q', u), ('S', u + 4))]
        for a, b in deps:
            assert pos[a] < pos[b], (a, b)
    return sched


SCHED = check(regular_schedule(), G * B)
SCHED_PAIR = check(parse("OPQ "
                         "OPQ"), 4)


def kernel(xa, ka, va, wqa, woa, xb, kb, vb, wqb, wob, go,
           out, dxa, dka, dva, dwqa, dwoa, dxb, dkb, dvb, dwqb, dwob,
           kbuf, vbuf, dkbuf, dvbuf, wqbuf, wobuf, dwqbuf, dwobuf,
           xbuf, gobuf, obuf, dxbuf,
           xc, gc, xt, gt, om, ol, dm, dl, q_s, do_s, oc, dqc, e_s,
           sem_in, sem_out, sem_act, sem_g):
    br = ((xa, ka, va, wqa, woa, dxa, dka, dva, dwqa, dwoa),
          (xb, kb, vb, wqb, wob, dxb, dkb, dvb, dwqb, dwob))

    def start_w(rr, hp, s):
        wq, wo = br[rr][3:5]
        cols = rows(hp * W, W, W)
        start(wq.at[:, cols], wqbuf.at[s], sem_in.at[s, 0])
        start(wo.at[cols, :], wobuf.at[s], sem_in.at[s, 1])

    def start_in(rr, hp, s):
        k, v = br[rr][1:3]
        start_w(rr, hp, s)
        start(k.at[:, pl.ds(hp * G, G)], kbuf.at[s], sem_in.at[s, 2])
        start(v.at[:, pl.ds(hp * G, G)], vbuf.at[s], sem_in.at[s, 3])

    def wait_out(s):
        for n, buf in enumerate((dkbuf, dvbuf, dwqbuf, dwobuf)):
            wait_for(buf.at[s], sem_out.at[s, n])

    def start_act_out(rr, which, rs, priority=0):
        dst, c0 = (out, rr * D) if which == 0 else (br[rr][5], 0)
        start((obuf, dxbuf)[which].at[rr, rs], dst.at[rs, pl.ds(c0, D)], sem_act.at[2 + which], priority)

    def kv_group(g, act):
        bs = pl.ds(2 * g, 2)
        act(ka.at[bs, pl.ds(0, G)], kbuf.at[0, bs], sem_g.at[g, 0])
        act(va.at[bs, pl.ds(0, G)], vbuf.at[0, bs], sem_g.at[g, 1])

    def x_group(g, act):
        rs = rows(2 * SQ * g, 2 * SQ, 16)
        act(xa.at[rs], xbuf.at[rs], sem_g.at[g, 2])
        act(go.at[rs, pl.ds(0, D)], gobuf.at[rs], sem_g.at[g, 3])

    def start_kv_step1(g):
        bs = pl.ds(2 * g, 2)
        start(ka.at[bs, pl.ds(G, G)], kbuf.at[1, bs], sem_in.at[1, 2])
        start(va.at[bs, pl.ds(G, G)], vbuf.at[1, bs], sem_in.at[1, 3])

    wait = lambda src, dst, sem: wait_for(dst, sem)

    def for_step(step, fn, lo=0, hi=NSTEPS):
        for rr in range(2):
            a, b = max(lo, rr * NS), min(hi, (rr + 1) * NS)
            if a < b:
                @pl.when(jnp.logical_and(step >= a, step < b))
                def _():
                    fn(rr, step - rr * NS)

    def natural(src, cmb, be):
        for p in range(0, SQ, 32):
            n_r = min(32, SQ - p)
            r1, r2 = rows(2 * be * SQ + p, n_r, 16), rows((2 * be + 1) * SQ + p, n_r, 16)
            ro = rows(be * SQ + p, n_r, 16)
            for c in range(2):
                f = lambda rr, d: src[rr, pl.ds(d * DP + c * 128, 128)]
                cs = combos(f(r1, 0), f(r2, 0), f(r1, 1), f(r2, 1), repack=True)
                for n in range(7):
                    cmb[2 * n + c, ro, :] = cs[n]
            for n, rr in ((14, r1), (15, r2)):
                cmb[n, ro, :] = (src[rr, pl.ds(2 * DP, DC)].astype(F32) + 0.0).astype(BF16)

    def transposed(src, cmt, c):
        base = [((8 * c + g) // 7) * 2 * SQ + ((8 * c + g) % 7) * 16 for g in range(8)]
        tile_t = lambda t, d: jnp.concatenate(
            [src[rows(r0 + t * SQ, 16, 16), pl.ds(d * 128, 128)] for r0 in base], axis=0).T
        for d in range(ND):
            z1, z2 = tile_t(0, d), tile_t(1, d)
            cs = combos(z1[:64], z2[:64], z1[64:], z2[64:], repack=True)
            for n in range(7):
                cmt[n, c, pl.ds(d * 64, 64), :] = cs[n]

    def make_stages(i, slot, first, pair_of):
        st, ov, dqv, wts = {}, {}, {}, {}
        prow = lambda be: rows(be * SQ, SQ, 16)
        split = lambda u: (u // 4, (u // 2) % 2, u % 2)
        getk = lambda p, t, j: kbuf[slot, 2 * pair_of(p) + t, j]
        getv = lambda p, t, j: vbuf[slot, 2 * pair_of(p) + t, j]
        getq = lambda p, t, j: q_s[j, t, prow(p), :]
        getdo = lambda p, t, j: do_s[j, t, prow(p), :]
        tiles = lambda n: jnp.concatenate([e_s[n, c] for c in range(NC)], axis=1)

        def store_tiles(n, val):
            for c in range(NC):
                e_s[n, c] = val[:, c * 128:(c + 1) * 128].astype(BF16)

        def weights(which):
            if not wts:
                wq, wo = wqbuf[slot], wobuf[slot]
                fq = lambda j, d: wq[d * DP:(d + 1) * DP, j * DH:(j + 1) * DH]
                fo = lambda j, d: wo[j * DH:(j + 1) * DH, d * DP:(d + 1) * DP]
                wts['q'] = combos(fq(0, 0), fq(0, 1), fq(1, 0), fq(1, 1)), wq[2 * DP:, :]
                wts['o'] = combos(fo(0, 0), fo(0, 1), fo(1, 0), fo(1, 1)), wo[:, 2 * DP:]
            return wts[which]

        def start_dkv(rr, hp, which, bs):
            src, dst = (dkbuf, dvbuf)[which], br[rr][6 + which]
            start(src.at[slot, bs], dst.at[bs, pl.ds(hp * G, G)], sem_out.at[slot, which])

        def start_dw(rr, hp):
            dwq, dwo = br[rr][8:10]
            cols = rows(hp * W, W, W)
            start(dwqbuf.at[slot], dwq.at[:, cols], sem_out.at[slot, 2])
            start(dwobuf.at[slot], dwo.at[cols, :], sem_out.at[slot, 3])

        def proj_in(p, cmb, which, dims, dst, mul):
            wc, wl = weights(which)
            get = lambda n: cmb[n, prow(pair_of(p)), :]
            rest = [dot(get(14 + t), wl, dims) for t in range(2)]
            m = [None] * 7
            for n in (OPQ if first else (2, 3, 0, 1, 4, 5, 6)):
                lhs = jnp.concatenate([get(2 * BORD[n]), get(2 * BORD[n] + 1)], axis=1)
                m[n] = dot(lhs, wc[n], dims)
            c = recombine(m)
            for t in range(2):
                for j in range(2):
                    val = c[2 * j + t] + rest[t][:, j * DH:(j + 1) * DH]
                    if mul is not None:
                        val = val * mul
                    dst[j, t, prow(p), :] = val.astype(BF16)

        def proj_out(p, vals, cmb, which, dims, macc, lacc, stage):
            wc, wl = weights(which)
            be = pair_of(p)
            ro = prow(be)
            z = [[vals.pop((p, t, j)) for j in range(2)] for t in range(2)]
            cs = combos(z[0][0], z[0][1], z[1][0], z[1][1]) + [z[0][1].astype(BF16), z[1][0].astype(BF16)]
            for n in range(9):
                cmb[n, ro, :] = cs[n]
            get = lambda n: cmb[n, ro, :]
            head = (lambda j: wl[j * DH:(j + 1) * DH, :]) if dims is NN else (lambda j: wl[:, j * DH:(j + 1) * DH])
            m = [None] * 7
            for n in (0, 3, 6, 4, 2, 1, 5):
                m[n] = dot(get(n), wc[BORD[n]], dims)
                if not first:
                    m[n] = m[n] + macc[n, ro, :]
                macc[n, ro, :] = m[n]
            c = None if first else recombine(m)
            for t, (n0, n1) in enumerate(((2, 7), (8, 3))):
                rest = dot(get(n0), head(0), dims) + dot(get(n1), head(1), dims)
                if not first:
                    rest = rest + lacc[t, ro, :]
                lacc[t, ro, :] = rest
                if not first:
                    row = jnp.concatenate([c[2 * t], c[2 * t + 1], rest], axis=1)
                    stage[i // NS, pl.ds((2 * be + t) * SQ, SQ), :] = row.astype(BF16)
            if not first:
                @pl.when(i == NSTEPS - 1)
                def _():
                    start_act_out(1, 0 if which == 'o' else 1, pl.ds(2 * be * SQ, 2 * SQ))

        def proj_w(cmb, cmt):
            m = [dot(jnp.concatenate([cmt[n, c] for c in range(NK)], axis=1), cmb[BORD[n]], NN)
                 for n in range(7)]
            c = recombine(m)
            top = jnp.concatenate([c[0], c[1]], axis=1)
            bot = jnp.concatenate([c[2], c[3]], axis=1)
            rs = [z[d * 64:(d + 1) * 64] for d in range(ND) for z in (top, bot)]
            return jnp.concatenate(rs, axis=0).astype(BF16)

        def S(u):
            s = dot(getq(*split(u)), getk(*split(u)), NT)
            e = jnp.exp2(s - jnp.max(s, axis=-1, keepdims=True))
            l = jnp.sum(e, axis=-1, keepdims=True)
            rcp = pl.reciprocal(l, approx=True)
            r = rcp * (2.0 - l * rcp)
            store_tiles(u % 4, e)
            st.setdefault(u, {}).update(e=None if first else e.astype(BF16), r=r,
                                        dor=(getdo(*split(u)).astype(F32) * r).astype(BF16))

        def P(u):
            st.setdefault(u, {})['dp'] = dot(getdo(*split(u)), getv(*split(u)), NT)

        def O(u):
            o = dot(tiles(u % 4) if first else st[u]['e'], getv(*split(u)), NN) * st[u]['r']
            st[u]['delta'] = jnp.sum(o * getdo(*split(u)).astype(F32), axis=-1, keepdims=True)
            ov[split(u)] = o

        def Q(u):
            ds = tiles(u % 4).astype(F32) * (st[u]['dp'] - st[u]['delta'])
            if first:
                store_tiles(4 + u % 4, ds)
                st[u]['ds'] = tiles(4 + u % 4)
            else:
                st[u]['ds'] = ds.astype(BF16)
            dqv[split(u)] = dot(st[u]['ds'], getk(*split(u)), NN) * (st[u]['r'] * SCALE)

        def kv_grad(u, lhs, rhs, which):
            p, t, j = split(u)
            dst, b = (dkbuf, dvbuf)[which], 2 * pair_of(p) + t
            if first:
                for c in range(NC):
                    dst[slot, b, j, pl.ds(c * 128, 128), :] = dot(lhs[:, c * 128:(c + 1) * 128], rhs, TN).astype(BF16)
            else:
                dst[slot, b, j] = dot(lhs, rhs, TN).astype(BF16)
                if u % 4 == 3:
                    for_step(i, lambda rr, hp: start_dkv(rr, hp, which, pl.ds(2 * p, 2)), lo=EARLY)

        def V(u):
            kv_grad(u, tiles(u % 4), st[u]['dor'], 1)

        def K(u):
            qr = (getq(*split(u)).astype(F32) * (st[u]['r'] * (1.0 / LOG2E))).astype(BF16)
            kv_grad(u, st[u]['ds'], qr, 0)

        def WO(_):
            dwobuf[slot] = proj_w(oc, gt).T

        def WQ(_):
            dwqbuf[slot] = proj_w(dqc, xt)

        def END(_):
            for which in range(2):
                for_step(i, lambda rr, hp: start_dkv(rr, hp, which, pl.ds(0, B)), hi=EARLY)
            for_step(i + 2, lambda rr, hp: start_in(rr, hp, slot))
            for_step(i, start_dw)

        nxt = lambda p: jnp.minimum(pair_of(p) + 1, NB - 1)
        tile = lambda p: jnp.minimum(pair_of(p), NK - 1)
        return dict(
            S=S, P=P, O=O, V=V, Q=Q, K=K, WO=WO, WQ=WQ, END=END,
            XQ=lambda p: proj_in(p, xc, 'q', NN, q_s, SCALE * LOG2E),
            XO=lambda p: proj_in(p, gc, 'o', NT, do_s, None),
            YO=lambda p: proj_out(p, ov, oc, 'o', NN, om, ol, obuf),
            YQ=lambda p: proj_out(p, dqv, dqc, 'q', NT, dm, dl, dxbuf),
            NX=lambda p: natural(xbuf, xc, nxt(p)),
            NG=lambda p: natural(gobuf, gc, nxt(p)),
            TX=lambda p: transposed(xbuf, xt, tile(p)),
            TG=lambda p: transposed(gobuf, gt, tile(p)))

    def first_step(i):
        @pl.when(i == 0)
        def _():
            x_group(0, wait)

        @pl.when(i == NS)
        def _():
            for which in range(2):
                start_act_out(0, which, pl.ds(0, T), priority=1)
            wait_for(xbuf, sem_act.at[0])
            wait_for(gobuf, sem_act.at[1])
            wait_for(kbuf.at[0], sem_in.at[0, 2])
            wait_for(vbuf.at[0], sem_in.at[0, 3])
            wait_out(0)
        natural(xbuf, xc, 0)
        natural(gobuf, gc, 0)
        wait_for(wqbuf.at[0], sem_in.at[0, 0])
        wait_for(wobuf.at[0], sem_in.at[0, 1])

        def pair(be, carry):
            @pl.when(i == 0)
            def _():
                kv_group(be, wait)

            @pl.when(jnp.logical_and(i == 0, be + 1 < NB))
            def _():
                x_group(be + 1, wait)

            @pl.when(jnp.logical_and(i == 0, be + 2 < NB))
            def _():
                kv_group(be + 2, start)

            @pl.when(jnp.logical_and(i == 0, be + 3 < NB))
            def _():
                x_group(be + 3, start)

            @pl.when(i == 0)
            def _():
                start_kv_step1(be)
            stages = make_stages(i, 0, True, lambda p: be)
            for name, idx in SCHED_PAIR:
                stages[name](idx)
            return carry
        lax.fori_loop(0, NB, pair, 0)

        stages = make_stages(i, 0, True, None)
        stages['WO'](0)
        stages['WQ'](0)

        @pl.when(i == 0)
        def _():
            start(xb, xbuf, sem_act.at[0], priority=1)
            start(go.at[:, pl.ds(D, D)], gobuf, sem_act.at[1], priority=1)
        stages['END'](0)

    def regular_step(i):
        slot = i % 2
        for n, buf in enumerate((wqbuf, wobuf, kbuf, vbuf)):
            wait_for(buf.at[slot], sem_in.at[slot, n])

        @pl.when(i >= 2)
        def _():
            wait_out(slot)
        stages = make_stages(i, slot, False, lambda p: p)
        for name, idx in SCHED:
            stages[name](idx)

    def branch(rr, carry):
        first_step(rr * NS)

        def body(j, c):
            regular_step(rr * NS + j)
            return c
        lax.fori_loop(1, NS, body, 0)
        return carry

    x_group(0, start)
    start_w(0, 0, 0)
    kv_group(0, start)
    x_group(1, start)
    kv_group(1, start)
    x_group(2, start)
    start_w(0, 1, 1)
    lax.fori_loop(0, 2, branch, 0)
    wait_out(0)
    wait_out(1)
    wait_for(obuf, sem_act.at[2])
    wait_for(dxbuf, sem_act.at[3])


def run_full(A_x, A_k_cache, A_v_cache, A_wq, A_wo, B_x, B_k_cache, B_v_cache, B_wq, B_wo, grad_out):
    hbm = pl.BlockSpec(memory_space=pl.ANY)
    sds = lambda *s: jax.ShapeDtypeStruct(s, BF16)
    grads = [sds(T, D), sds(B, H, SK, DH), sds(B, H, SK, DH), sds(D, H * DH), sds(H * DH, D)]
    vmem = pltpu.VMEM
    scratch = (
        [vmem((2, B, G, SK, DH), BF16)] * 4
        + [vmem((2, D, W), BF16), vmem((2, W, D), BF16)] * 2
        + [vmem((T, D), BF16)] * 2 + [vmem((2, T, D), BF16)] * 2
        + [vmem((16, TH, 128), BF16)] * 2 + [vmem((7, NK, DHF, 128), BF16)] * 2
        + [vmem((7, TH, DP), F32), vmem((2, TH, DC), F32)] * 2
        + [vmem((2, 2, TH, DH), BF16)] * 2 + [vmem((9, TH, DH), BF16)] * 2
        + [vmem((8, NC, SQ, 128), BF16)]
        + [pltpu.SemaphoreType.DMA((2, 4)), pltpu.SemaphoreType.DMA((2, 4)),
           pltpu.SemaphoreType.DMA((4,)), pltpu.SemaphoreType.DMA((NB, 4))])
    outs = list(pl.pallas_call(
        kernel,
        in_specs=[hbm] * 11,
        out_specs=[hbm] * 11,
        out_shape=[sds(T, 2 * D)] + grads + grads,
        scratch_shapes=scratch,
        compiler_params=pltpu.CompilerParams(vmem_limit_bytes=100 * 2**20, disable_bounds_checks=True,
                                             disable_semaphore_checks=True),
        name=NAME,
    )(A_x.reshape(T, D), A_k_cache, A_v_cache, A_wq, A_wo,
      B_x.reshape(T, D), B_k_cache, B_v_cache, B_wq, B_wo, grad_out.reshape(T, 2 * D)))
    outs[0] = outs[0].reshape(B, SQ, 2 * D)
    outs[1] = outs[1].reshape(B, SQ, D)
    outs[6] = outs[6].reshape(B, SQ, D)
    return tuple(outs)


@jax.jit
def pallas_concat_heads__gqa_block_cached__gqa_block_cached__near_ridge_kernel(
    A_x: jax.Array,
    A_k_cache: jax.Array,
    A_v_cache: jax.Array,
    A_wq: jax.Array,
    A_wo: jax.Array,
    B_x: jax.Array,
    B_k_cache: jax.Array,
    B_v_cache: jax.Array,
    B_wq: jax.Array,
    B_wo: jax.Array,
    grad_out: jax.Array,
):
    return run_full(A_x, A_k_cache, A_v_cache, A_wq, A_wo, B_x, B_k_cache, B_v_cache, B_wq, B_wo, grad_out)
```

```python
import jax
import jax.numpy as jnp
from jax import lax
from jax.experimental import pallas as pl
from jax.experimental.pallas import tpu as pltpu

NAME = "concat_heads_gqa_fwd_bwd"
B, SQ, D, H, SK, DH = 16, 112, 640, 32, 512, 128
T = B * SQ
TH = T // 2
G = 2
W = G * DH
NS = H // G
NSTEPS = 2 * NS
EARLY = NSTEPS - 2
NB = B // 2
NK = TH // 128
ND = D // 128
NC = SK // 128
DP = 256
DC = D - 2 * DP
DHF = D // 2
F32, BF16 = jnp.float32, jnp.bfloat16
NN = (((1,), (0,)), ((), ()))
NT = (((1,), (1,)), ((), ()))
TN = (((0,), (0,)), ((), ()))
SCALE = DH ** -0.5
LOG2E = 1.4426950408889634
BORD = (0, 2, 6, 5, 3, 4, 1)


def combos(z11, z12, z21, z22, repack=False):
    f11, f12, f21, f22 = (z.astype(F32) for z in (z11, z12, z21, z22))
    if repack:
        z11, z22 = f11 + 0.0, f22 + 0.0
    return [c.astype(BF16) for c in
            (f11 + f22, f21 + f22, z11, z22, f11 + f12, f21 - f11, f12 - f22)]


def recombine(m):
    return (m[0] + m[3] - m[4] + m[6], m[2] + m[4], m[1] + m[3], m[0] - m[1] + m[2] + m[5])


def dot(a, b, dims):
    return lax.dot_general(a, b, dims, preferred_element_type=F32)


def rows(start, size, align):
    return pl.ds(start if isinstance(start, int) else pl.multiple_of(start, align), size)


def start(src, dst, sem, priority=0):
    pltpu.make_async_copy(src, dst, sem).start(priority=priority)


def wait_for(buf, sem):
    pltpu.make_async_copy(buf, buf, sem).wait()


def parse(items):
    out = []
    for z in items.split():
        name = z.rstrip('0123456789')
        out.append((name, int(z[len(name):])))
    return out


def check(sched, n_units):
    pos = {it: n for n, it in enumerate(sched)}
    assert len(pos) == len(sched)
    for u in range(n_units):
        p = u // 4
        deps = [(('XQ', p), ('S', u)), (('XO', p), ('S', u)), (('XO', p), ('P', u)), (('S', u), ('O', u)),
                (('S', u), ('V', u)), (('O', u), ('Q', u)), (('P', u), ('Q', u)), (('Q', u), ('K', u)),
                (('O', u), ('YO', p)), (('Q', u), ('YQ', p))]
        if n_units > 4:
            deps += [(('Y' + w, p), (z + w, n)) for w in 'OQ' for z in 'WZ' for n in range(7)]
            if u % 4 < 3:
                deps += [(('V', u), ('V', 4 * p + 3)), (('K', u), ('K', 4 * p + 3))]
        else:
            deps += [(('XQ', 0), ('NX', 0)), (('XO', 0), ('NG', 0))]
        if u + 4 < n_units:
            deps += [(('V', u), ('S', u + 4)), (('Q', u), ('S', u + 4))]
        for a, b in deps:
            assert pos[a] < pos[b], (a, b)
    return sched


SCHED = check(parse(
    "XQ0 XO0 S0 XQ1 S1 XO1 O0 V0 P0 XQ2 S2 O1 Q0 V1 K0 P1 S3 O2 Q1 V2 K1 P2 S4 O3 Q2 V3 K2 P3 S5 O4 Q3 V4 "
    "K3 P4 XO2 S6 O5 Q4 V5 YO0 K4 P5 S7 O6 Q5 V6 K5 P6 YQ0 S8 O7 Q6 V7 XQ3 K6 P7 S9 O8 Q7 V8 K7 P8 O9 XO3 "
    "S10 Q8 V9 YO1 K8 P9 S11 O10 Q9 V10 K9 P10 S12 O11 YQ1 Q10 V11 K10 P11 XQ4 S13 O12 Q11 V12 K11 P12 "
    "XO4 S14 O13 Q12 V13 YO2 K12 P13 S15 O14 Q13 V14 K13 P14 YQ2 S16 O15 Q14 V15 XQ5 K14 P15 S17 O16 Q15 "
    "V16 K15 P16 XO5 S18 O17 Q16 V17 YO3 K16 P17 S19 O18 Q17 V18 K17 P18 YQ3 S20 O19 Q18 V19 XQ6 K18 P19 "
    "S21 O20 Q19 V20 K19 P20 XO6 S22 O21 Q20 V21 YO4 K20 P21 S23 O22 Q21 V22 K21 P22 YQ4 S24 O23 Q22 V23 "
    "XQ7 K22 P23 S25 O24 Q23 V24 K23 XO7 P24 S26 O25 Q24 V25 YO5 K24 P25 S27 O26 Q25 V26 K25 P26 S28 O27 "
    "Q26 V27 K26 YQ5 P27 YO6 S29 O28 Q27 V28 K27 P28 S30 O29 Q28 V29 K28 P29 S31 O30 Q29 V30 K29 P30 YQ6 "
    "O31 Q30 V31 K30 P31 YO7 WO1 Q31 K31 WO0 ZO0 ZO1 ZO2 ZO3 YQ7 ZO4 WO2 ZO5 ZO6 ZQ0 WO3 ZQ1 ZQ2 WO4 ZQ4 "
    "WO5 ZQ5 ZQ6 ZQ3 WO6 WQ0 WQ1 WQ3 WQ2 WQ4 WQ5 WQ6 END0 "), G * B)
SCHED_PAIR = check(parse(
    "XQ0 XO0 TX0 S0 S1 S2 O0 S3 P0 O1 P1 NX0 V1 V0 P2 Q0 O2 K0 Q1 P3 O3 K1 TG0 V3 V2 YO0 Q2 Q3 K2 K3 NG0 "
    "YQ0 "), 4)
SCHED_W = parse(
    "WO0 ZO0 ZO2 ZO1 WO1 ZO3 WO2 ZO4 ZO5 WO3 ZO6 WO4 ZQ0 ZQ1 ZQ2 WO5 ZQ3 ZQ4 WO6 ZQ5 ZQ6 WQ0 WQ1 WQ2 WQ3 "
    "WQ4 WQ5 WQ6 ")
X_ORDER, X_ORDER_FIRST, Y_ORDER = (6, 4, 2, 5, 1, 0, 3), (1, 5, 4, 0, 2, 3, 6), (1, 3, 5, 4, 2, 6, 0)
TIE_LAG = 2


def kernel(xa, ka, va, wqa, woa, xb, kb, vb, wqb, wob, go,
           out, dxa, dka, dva, dwqa, dwoa, dxb, dkb, dvb, dwqb, dwob,
           kbuf, vbuf, dkbuf, dvbuf, wqbuf, wobuf, dwqbuf, dwobuf,
           xbuf, gobuf, obuf, dxbuf, obl, dxbl,
           xc, gc, xt, gt, om, ol, dm, dl, q_s, do_s, oc, dqc, e_s,
           sem_in, sem_out, sem_act, sem_g):
    br = ((xa, ka, va, wqa, woa, dxa, dka, dva, dwqa, dwoa),
          (xb, kb, vb, wqb, wob, dxb, dkb, dvb, dwqb, dwob))

    def start_w(rr, hp, s):
        wq, wo = br[rr][3:5]
        cols = rows(hp * W, W, W)
        start(wq.at[:, cols], wqbuf.at[s], sem_in.at[s, 0])
        start(wo.at[cols, :], wobuf.at[s], sem_in.at[s, 1])

    def start_in(rr, hp, s):
        k, v = br[rr][1:3]
        start_w(rr, hp, s)
        start(k.at[:, pl.ds(hp * G, G)], kbuf.at[s], sem_in.at[s, 2])
        start(v.at[:, pl.ds(hp * G, G)], vbuf.at[s], sem_in.at[s, 3])

    def wait_out(s):
        for n, buf in enumerate((dkbuf, dvbuf, dwqbuf, dwobuf)):
            wait_for(buf.at[s], sem_out.at[s, n])

    def start_act_out(rr, which, rs, priority=0):
        dst, c0 = (out, rr * D) if which == 0 else (br[rr][5], 0)
        start((obuf, dxbuf)[which].at[rr, rs], dst.at[rs, pl.ds(c0, 2 * DP)], sem_act.at[2 + which], priority)

    def start_act_rest(rr, which, priority=0):
        dst, c0 = (out, rr * D) if which == 0 else (br[rr][5], 0)
        start((obl, dxbl)[which].at[rr], dst.at[:, pl.ds(c0 + 2 * DP, DC)], sem_act.at[4 + which], priority)

    def kv_group(g, act):
        bs = pl.ds(2 * g, 2)
        act(ka.at[bs, pl.ds(0, G)], kbuf.at[0, bs], sem_g.at[g, 0])
        act(va.at[bs, pl.ds(0, G)], vbuf.at[0, bs], sem_g.at[g, 1])

    def x_group(g, act):
        rs = rows(2 * SQ * g, 2 * SQ, 16)
        act(xa.at[rs], xbuf.at[rs], sem_g.at[g, 2])
        act(go.at[rs, pl.ds(0, D)], gobuf.at[rs], sem_g.at[g, 3])

    def start_kv_step1(g):
        bs = pl.ds(2 * g, 2)
        start(ka.at[bs, pl.ds(G, G)], kbuf.at[1, bs], sem_in.at[1, 2])
        start(va.at[bs, pl.ds(G, G)], vbuf.at[1, bs], sem_in.at[1, 3])

    wait = lambda src, dst, sem: wait_for(dst, sem)

    def for_step(step, fn, lo=0, hi=NSTEPS):
        for rr in range(2):
            a, b = max(lo, rr * NS), min(hi, (rr + 1) * NS)
            if a < b:
                @pl.when(jnp.logical_and(step >= a, step < b))
                def _():
                    fn(rr, step - rr * NS)

    def natural(src, cmb, be):
        for p in range(0, SQ, 32):
            n_r = min(32, SQ - p)
            r1, r2 = rows(2 * be * SQ + p, n_r, 16), rows((2 * be + 1) * SQ + p, n_r, 16)
            ro = rows(be * SQ + p, n_r, 16)
            for c in range(2):
                f = lambda rr, d: src[rr, pl.ds(d * DP + c * 128, 128)]
                cs = combos(f(r1, 0), f(r2, 0), f(r1, 1), f(r2, 1), repack=True)
                for n in range(7):
                    cmb[2 * n + c, ro, :] = cs[n]
            for n, rr in ((14, r1), (15, r2)):
                cmb[n, ro, :] = (src[rr, pl.ds(2 * DP, DC)].astype(F32) + 0.0).astype(BF16)

    def transposed(src, cmt, c):
        base = [((8 * c + g) // 7) * 2 * SQ + ((8 * c + g) % 7) * 16 for g in range(8)]
        tile_t = lambda t, d: jnp.concatenate(
            [src[rows(r0 + t * SQ, 16, 16), pl.ds(d * 128, 128)] for r0 in base], axis=0).T
        for d in range(ND):
            z1, z2 = tile_t(0, d), tile_t(1, d)
            cs = combos(z1[:64], z2[:64], z1[64:], z2[64:], repack=True)
            for n in range(7):
                cmt[n, c, pl.ds(d * 64, 64), :] = cs[n]

    def make_stages(i, slot, first, pair_of):
        st, ov, dqv, wts = {}, {}, {}, {}
        pending = []
        zero = None if first else (i // (2 * NSTEPS)).astype(F32)
        prow = lambda be: rows(be * SQ, SQ, 16)
        split = lambda u: (u // 4, (u // 2) % 2, u % 2)
        getk = lambda p, t, j: kbuf[slot, 2 * pair_of(p) + t, j]
        getv = lambda p, t, j: vbuf[slot, 2 * pair_of(p) + t, j]
        getq = lambda p, t, j: q_s[j, t, prow(p), :]
        getdo = lambda p, t, j: do_s[j, t, prow(p), :]
        tiles = lambda n: jnp.concatenate([e_s[n, c] for c in range(NC)], axis=1)

        def store_tiles(n, val):
            for c in range(NC):
                e_s[n, c] = val[:, c * 128:(c + 1) * 128].astype(BF16)

        def weights(which):
            if not wts:
                wq, wo = wqbuf[slot], wobuf[slot]
                fq = lambda j, d: wq[d * DP:(d + 1) * DP, j * DH:(j + 1) * DH]
                fo = lambda j, d: wo[j * DH:(j + 1) * DH, d * DP:(d + 1) * DP]
                wts['q'] = combos(fq(0, 0), fq(0, 1), fq(1, 0), fq(1, 1)), wq[2 * DP:, :]
                wts['o'] = combos(fo(0, 0), fo(0, 1), fo(1, 0), fo(1, 1)), wo[:, 2 * DP:]
            return wts[which]

        def start_dkv(rr, hp, which, bs):
            src, dst = (dkbuf, dvbuf)[which], br[rr][6 + which]
            start(src.at[slot, bs], dst.at[bs, pl.ds(hp * G, G)], sem_out.at[slot, which])

        def start_dw(rr, hp):
            dwq, dwo = br[rr][8:10]
            cols = rows(hp * W, W, W)
            start(dwqbuf.at[slot], dwq.at[:, cols], sem_out.at[slot, 2])
            start(dwobuf.at[slot], dwo.at[cols, :], sem_out.at[slot, 3])

        def proj_in(p, cmb, which, dims, dst, mul):
            wc, wl = weights(which)
            get = lambda n: cmb[n, prow(pair_of(p)), :]
            rest = [dot(get(14 + t), wl, dims) for t in range(2)]
            m = [None] * 7
            for n in (X_ORDER_FIRST if first else X_ORDER):
                lhs = jnp.concatenate([get(2 * BORD[n]), get(2 * BORD[n] + 1)], axis=1)
                m[n] = dot(lhs, wc[n], dims)
            c = recombine(m)
            for t in range(2):
                for j in range(2):
                    val = c[2 * j + t] + rest[t][:, j * DH:(j + 1) * DH]
                    if mul is not None:
                        val = val * mul
                    dst[j, t, prow(p), :] = val.astype(BF16)

        def proj_out(p, vals, cmb, which, dims, macc, stage):
            wc, _ = weights(which)
            be = pair_of(p)
            ro = prow(be)
            z = [[vals.pop((p, t, j)) for j in range(2)] for t in range(2)]
            cs = combos(z[0][0], z[0][1], z[1][0], z[1][1])
            for n in range(7):
                cmb[n, ro, :] = cs[n]
            m = [None] * 7
            for n in Y_ORDER:
                m[n] = dot(cmb[n, ro, :], wc[BORD[n]], dims)
                if not first:
                    m[n] = m[n] + macc[n, ro, :]
                macc[n, ro, :] = m[n]
            if not first:
                c = recombine(m)
                for t in range(2):
                    row = jnp.concatenate([c[2 * t], c[2 * t + 1]], axis=1)
                    stage[i // NS, pl.ds((2 * be + t) * SQ, SQ), :] = row.astype(BF16)

                @pl.when(i == NSTEPS - 1)
                def _():
                    start_act_out(1, 0 if which == 'o' else 1, pl.ds(2 * be * SQ, 2 * SQ))

        zw, zm, wm = {}, {0: {}, 1: {}}, {0: {}, 1: {}}
        def proj_rest(which, n):
            cmb, lacc, stage = ((oc, ol, obl), (dqc, dl, dxbl))[which]
            if which not in zw:
                wt = wqbuf[slot, 2 * DP:, :] if which else wobuf[slot, :, 2 * DP:].T
                blk = lambda j, d: wt[64 * d:64 * d + 64, j * DH:(j + 1) * DH]
                zw[which] = combos(blk(0, 0), blk(0, 1), blk(1, 0), blk(1, 1))
            m = dot(zw[which][BORD[n]], cmb[n], NT)
            if not first:
                m = m + lacc[n]
            lacc[n] = zm[which][n] = m
            if len(zm[which]) == 7 and not first:
                cl = recombine(zm[which])
                for t in range(2):
                    zt = jnp.concatenate([cl[2 * t], cl[2 * t + 1]], axis=0).astype(BF16).T
                    a = zt[112:128].astype(F32)
                    for c in range(1, NK):
                        a = a + zt[c * 128 + 112:c * 128 + 128].astype(F32)
                    pending.append([TIE_LAG, a])
                    for be in range(NB):
                        stage[i // NS, pl.ds((2 * be + t) * SQ, SQ), :] = zt[be * SQ:(be + 1) * SQ]

                @pl.when(i == NSTEPS - 1)
                def _():
                    start_act_rest(1, which)

        def proj_w(which, n):
            cmb, cmt = ((oc, gt), (dqc, xt))[which]
            rhs = cmb[BORD[n]]
            due = [a for a in pending if a[0] <= 0]
            for a in pending:
                a[0] -= 1
            if due:
                top = rhs[:16].astype(F32)
                for a in due:
                    pending.remove(a)
                    top = top + a[1] * zero
                rhs = jnp.concatenate([top.astype(BF16), rhs[16:]], axis=0)
            wm[which][n] = dot(jnp.concatenate([cmt[n, c] for c in range(NK)], axis=1), rhs, NN)
            if len(wm[which]) == 7:
                c = recombine(wm[which])
                top = jnp.concatenate([c[0], c[1]], axis=1)
                bot = jnp.concatenate([c[2], c[3]], axis=1)
                rs = [z[d * 64:(d + 1) * 64] for d in range(ND) for z in (top, bot)]
                res = jnp.concatenate(rs, axis=0).astype(BF16)
                if which:
                    dwqbuf[slot] = res
                else:
                    dwobuf[slot] = res.T

        def S(u):
            s = dot(getq(*split(u)), getk(*split(u)), NT)
            e = jnp.exp2(s - jnp.max(s, axis=-1, keepdims=True))
            l = jnp.sum(e, axis=-1, keepdims=True)
            rcp = pl.reciprocal(l, approx=True)
            r = rcp * (2.0 - l * rcp)
            store_tiles(u % 4, e)
            st.setdefault(u, {}).update(e=None if first else e.astype(BF16), r=r,
                                        dor=(getdo(*split(u)).astype(F32) * r).astype(BF16))

        def P(u):
            st.setdefault(u, {})['dp'] = dot(getdo(*split(u)), getv(*split(u)), NT)

        def O(u):
            o = dot(tiles(u % 4) if first else st[u]['e'], getv(*split(u)), NN) * st[u]['r']
            st[u]['delta'] = jnp.sum(o * getdo(*split(u)).astype(F32), axis=-1, keepdims=True)
            ov[split(u)] = o

        def Q(u):
            ds = tiles(u % 4).astype(F32) * (st[u]['dp'] - st[u]['delta'])
            if first:
                store_tiles(4 + u % 4, ds)
                st[u]['ds'] = tiles(4 + u % 4)
            else:
                st[u]['ds'] = ds.astype(BF16)
            dqv[split(u)] = dot(st[u]['ds'], getk(*split(u)), NN) * (st[u]['r'] * SCALE)

        def kv_grad(u, lhs, rhs, which):
            p, t, j = split(u)
            dst, b = (dkbuf, dvbuf)[which], 2 * pair_of(p) + t
            if first:
                for c in range(NC):
                    dst[slot, b, j, pl.ds(c * 128, 128), :] = dot(lhs[:, c * 128:(c + 1) * 128], rhs, TN).astype(BF16)
            else:
                dst[slot, b, j] = dot(lhs, rhs, TN).astype(BF16)
                if u % 4 == 3:
                    for_step(i, lambda rr, hp: start_dkv(rr, hp, which, pl.ds(2 * p, 2)), lo=EARLY)

        def V(u):
            kv_grad(u, tiles(u % 4), st[u]['dor'], 1)

        def K(u):
            qr = (getq(*split(u)).astype(F32) * (st[u]['r'] * (1.0 / LOG2E))).astype(BF16)
            kv_grad(u, st[u]['ds'], qr, 0)

        def END(_):
            for which in range(2):
                for_step(i, lambda rr, hp: start_dkv(rr, hp, which, pl.ds(0, B)), hi=EARLY)
            for_step(i + 2, lambda rr, hp: start_in(rr, hp, slot))
            for_step(i, start_dw)

        nxt = lambda p: jnp.minimum(pair_of(p) + 1, NB - 1)
        tile = lambda p: jnp.minimum(pair_of(p), NK - 1)
        return dict(
            S=S, P=P, O=O, V=V, Q=Q, K=K, END=END,
            WO=lambda n: proj_w(0, n), WQ=lambda n: proj_w(1, n), ZO=lambda n: proj_rest(0, n), ZQ=lambda n: proj_rest(1, n),
            XQ=lambda p: proj_in(p, xc, 'q', NN, q_s, SCALE * LOG2E),
            XO=lambda p: proj_in(p, gc, 'o', NT, do_s, None),
            YO=lambda p: proj_out(p, ov, oc, 'o', NN, om, obuf),
            YQ=lambda p: proj_out(p, dqv, dqc, 'q', NT, dm, dxbuf),
            NX=lambda p: natural(xbuf, xc, nxt(p)),
            NG=lambda p: natural(gobuf, gc, nxt(p)),
            TX=lambda p: transposed(xbuf, xt, tile(p)),
            TG=lambda p: transposed(gobuf, gt, tile(p)))

    def first_step(i):
        @pl.when(i == 0)
        def _():
            x_group(0, wait)

        @pl.when(i == NS)
        def _():
            for which in range(2):
                start_act_out(0, which, pl.ds(0, T), priority=1)
                start_act_rest(0, which, priority=1)
            wait_for(xbuf, sem_act.at[0])
            wait_for(gobuf, sem_act.at[1])
            wait_for(kbuf.at[0], sem_in.at[0, 2])
            wait_for(vbuf.at[0], sem_in.at[0, 3])
            wait_out(0)
        natural(xbuf, xc, 0)
        natural(gobuf, gc, 0)
        wait_for(wqbuf.at[0], sem_in.at[0, 0])
        wait_for(wobuf.at[0], sem_in.at[0, 1])

        def pair(be, carry):
            @pl.when(i == 0)
            def _():
                kv_group(be, wait)

            @pl.when(jnp.logical_and(i == 0, be + 1 < NB))
            def _():
                x_group(be + 1, wait)

            @pl.when(jnp.logical_and(i == 0, be + 2 < NB))
            def _():
                kv_group(be + 2, start)

            @pl.when(jnp.logical_and(i == 0, be + 3 < NB))
            def _():
                x_group(be + 3, start)

            @pl.when(i == 0)
            def _():
                start_kv_step1(be)
            stages = make_stages(i, 0, True, lambda p: be)
            for name, idx in SCHED_PAIR:
                stages[name](idx)
            return carry
        lax.fori_loop(0, NB, pair, 0)

        stages = make_stages(i, 0, True, None)
        for name, idx in SCHED_W:
            stages[name](idx)

        @pl.when(i == 0)
        def _():
            start(xb, xbuf, sem_act.at[0], priority=1)
            start(go.at[:, pl.ds(D, D)], gobuf, sem_act.at[1], priority=1)
        stages['END'](0)

    def regular_step(i):
        slot = i % 2
        for n, buf in enumerate((wqbuf, wobuf, kbuf, vbuf)):
            wait_for(buf.at[slot], sem_in.at[slot, n])

        @pl.when(i >= 2)
        def _():
            wait_out(slot)
        stages = make_stages(i, slot, False, lambda p: p)
        for name, idx in SCHED:
            stages[name](idx)

    def branch(rr, carry):
        first_step(rr * NS)

        def body(j, c):
            regular_step(rr * NS + j)
            return c
        lax.fori_loop(1, NS, body, 0)
        return carry

    x_group(0, start)
    start_w(0, 0, 0)
    kv_group(0, start)
    x_group(1, start)
    kv_group(1, start)
    x_group(2, start)
    start_w(0, 1, 1)
    lax.fori_loop(0, 2, branch, 0)
    wait_out(0)
    wait_out(1)
    wait_for(obuf, sem_act.at[2])
    wait_for(dxbuf, sem_act.at[3])
    wait_for(obl, sem_act.at[4])
    wait_for(dxbl, sem_act.at[5])


def run_full(A_x, A_k_cache, A_v_cache, A_wq, A_wo, B_x, B_k_cache, B_v_cache, B_wq, B_wo, grad_out):
    hbm = pl.BlockSpec(memory_space=pl.ANY)
    sds = lambda *s: jax.ShapeDtypeStruct(s, BF16)
    grads = [sds(T, D), sds(B, H, SK, DH), sds(B, H, SK, DH), sds(D, H * DH), sds(H * DH, D)]
    vmem = pltpu.VMEM
    scratch = (
        [vmem((2, B, G, SK, DH), BF16)] * 4
        + [vmem((2, D, W), BF16), vmem((2, W, D), BF16)] * 2
        + [vmem((T, D), BF16)] * 2
        + [vmem((2, T, 2 * DP), BF16)] * 2 + [vmem((2, T, DC), BF16)] * 2
        + [vmem((16, TH, 128), BF16)] * 2 + [vmem((7, NK, DHF, 128), BF16)] * 2
        + [vmem((7, TH, DP), F32), vmem((7, 64, TH), F32)] * 2
        + [vmem((2, 2, TH, DH), BF16)] * 2 + [vmem((7, TH, DH), BF16)] * 2
        + [vmem((8, NC, SQ, 128), BF16)]
        + [pltpu.SemaphoreType.DMA((2, 4)), pltpu.SemaphoreType.DMA((2, 4)),
           pltpu.SemaphoreType.DMA((6,)), pltpu.SemaphoreType.DMA((NB, 4))])
    outs = list(pl.pallas_call(
        kernel,
        in_specs=[hbm] * 11,
        out_specs=[hbm] * 11,
        out_shape=[sds(T, 2 * D)] + grads + grads,
        scratch_shapes=scratch,
        compiler_params=pltpu.CompilerParams(vmem_limit_bytes=100 * 2**20, disable_bounds_checks=True,
                                             disable_semaphore_checks=True),
        name=NAME,
    )(A_x.reshape(T, D), A_k_cache, A_v_cache, A_wq, A_wo,
      B_x.reshape(T, D), B_k_cache, B_v_cache, B_wq, B_wo, grad_out.reshape(T, 2 * D)))
    outs[0] = outs[0].reshape(B, SQ, 2 * D)
    outs[1] = outs[1].reshape(B, SQ, D)
    outs[6] = outs[6].reshape(B, SQ, D)
    return tuple(outs)


@jax.jit
def pallas_concat_heads__gqa_block_cached__gqa_block_cached__near_ridge_kernel(
    A_x: jax.Array,
    A_k_cache: jax.Array,
    A_v_cache: jax.Array,
    A_wq: jax.Array,
    A_wo: jax.Array,
    B_x: jax.Array,
    B_k_cache: jax.Array,
    B_v_cache: jax.Array,
    B_wq: jax.Array,
    B_wo: jax.Array,
    grad_out: jax.Array,
):
    return run_full(A_x, A_k_cache, A_v_cache, A_wq, A_wo, B_x, B_k_cache, B_v_cache, B_wq, B_wo, grad_out)
```
